```python
import os as _os
_os.environ.setdefault("JAX_PLATFORMS", "cpu")
import jax
import jax.numpy as jnp

def _softmax(x, axis=-1):
    return jax.nn.softmax(x, axis=axis)
def _gelu(x):
    return jax.nn.gelu(x, approximate=True)
def _silu(x):
    return jax.nn.silu(x)
def _sigmoid(x):
    return jax.nn.sigmoid(x)
def _layernorm(x, axis=-1, eps=1e-5):
    m = jnp.mean(x, axis=axis, keepdims=True)
    v = jnp.var(x, axis=axis, keepdims=True)
    return (x - m) / jnp.sqrt(v + eps)
def _scatter_add(tgt, idx, src, axis=0):
    return tgt.at[idx].add(src)
def _segment_sum(src, seg, n):
    return jax.ops.segment_sum(src, seg, n)
class _Rng:
    def __init__(self, key):
        self._k = key
    def _next(self):
        self._k, sub = jax.random.split(self._k)
        return sub
    def normal(self, shape):
        return jax.random.normal(self._next(), shape, dtype=jnp.bfloat16)
    def randint(self, lo, hi, shape):
        return jax.random.randint(self._next(), shape, lo, hi, dtype=jnp.int32)
    def uniform(self, shape, lo=0.0, hi=1.0):
        return jax.random.uniform(self._next(), shape, jnp.bfloat16, lo, hi)
    def permutation(self, n):
        return jax.random.permutation(self._next(), n)


kernel_name = 'interleave_layers__linear_kernel_hedgehog__ssm_conv_s4__prompt'

def setup_inputs():
    _rng = _Rng(jax.random.key(int.from_bytes(__import__("os").urandom(4), "little")))
    _w = (lambda a: (lambda t: t.astype(jnp.bfloat16) if jnp.issubdtype(t.dtype, jnp.floating) else t)(jnp.asarray(a)))
    def _A_setup():
        B, S, D, H = 1, 2048, 512, 32
        Dh = D // H
        return {
            "x": _w((lambda *s: _rng.normal(s) * 0.05)(B, S, D)),
            "wqkv": _w((lambda *s: _rng.normal(s) * 0.4)(D, 3 * D)),
            "w_phi": _w((lambda *s: _rng.normal(s) * 0.4)(H, Dh, Dh) * (Dh ** -0.5)),
            "wo": _w((lambda *s: _rng.normal(s) * 0.05)(D, D)),
        }
    _A_in = _A_setup()

    def _B_setup():
        B, L, D, N = 1, 2048, 512, 128
        A_re = -jnp.exp((lambda *s: _rng.normal(s) * 0.2)(D, N))
        A_im = jnp.pi * (lambda *s: _rng.normal(s) * 0.2)(D, N)
        B_re = (lambda *s: _rng.normal(s) * 0.2)(D, N)
        B_im = (lambda *s: _rng.normal(s) * 0.2)(D, N)
        C_re = (lambda *s: _rng.normal(s) * 0.2)(D, N)
        C_im = (lambda *s: _rng.normal(s) * 0.2)(D, N)
        log_dt = (lambda *s: _rng.normal(s) * 0.2)(D) * 0.5 - 4.0
        Dskip = (lambda *s: _rng.normal(s) * 0.2)(D)
        return {
            "u": _w((lambda *s: _rng.normal(s) * 0.05)(B, L, D)),
            "A_re": _w(A_re),
            "A_im": _w(A_im),
            "B_re": _w(B_re),
            "B_im": _w(B_im),
            "C_re": _w(C_re),
            "C_im": _w(C_im),
            "log_dt": _w(log_dt),
            "Dskip": _w(Dskip),
        }
    _B_in = _B_setup()

    return {
        "A_x": _A_in["x"],
        "A_wqkv": _A_in["wqkv"],
        "A_w_phi": _A_in["w_phi"],
        "A_wo": _A_in["wo"],
        "B_u": _B_in["u"],
        "B_A_re": _B_in["A_re"],
        "B_A_im": _B_in["A_im"],
        "B_B_re": _B_in["B_re"],
        "B_B_im": _B_in["B_im"],
        "B_C_re": _B_in["C_re"],
        "B_C_im": _B_in["C_im"],
        "B_log_dt": _B_in["log_dt"],
        "B_Dskip": _B_in["Dskip"],
    }

def reference(A_x, A_wqkv, A_w_phi, A_wo, B_u, B_A_re, B_A_im, B_B_re, B_B_im, B_C_re, B_C_im, B_log_dt, B_Dskip):
    def _A_ref(x, wqkv, w_phi, wo):
        B, S, D = x.shape
        H = 32; Dh = D // H
        qkv = (lambda x, *d: x.transpose(*d))((x @ wqkv).reshape(B, S, 3, H, Dh), 2, 0, 3, 1, 4)
        q, k, v = qkv[0], qkv[1], qkv[2]
        pq = jnp.einsum("bhsd,hdf->bhsf", q, w_phi)
        pk = jnp.einsum("bhsd,hdf->bhsf", k, w_phi)
        phi_q = jnp.concatenate([_softmax(pq, axis=-1), _softmax(-pq, axis=-1)], axis=-1)
        phi_k = jnp.concatenate([_softmax(pk, axis=-1), _softmax(-pk, axis=-1)], axis=-1)
        kv = jnp.einsum("bhsf,bhsd->bhfd", phi_k, v)
        z  = jnp.einsum("bhsf->bhf", phi_k)
        num = jnp.einsum("bhqf,bhfd->bhqd", phi_q, kv)
        den = jnp.einsum("bhqf,bhf->bhq", phi_q, z)[..., None] + 1e-6
        o = num / den
        return (lambda x, *d: x.transpose(*d))(o, 0, 2, 1, 3).reshape(B, S, D) @ wo

    def _B_ref(u, A_re, A_im, B_re, B_im, C_re, C_im, log_dt, Dskip):
        Bsz, L, D = u.shape
        dt = jnp.exp(log_dt)[:, None]
        A = A_re + 1j * A_im
        Bc = B_re + 1j * B_im
        Cc = C_re + 1j * C_im
        logdA = dt * A
        dB = dt * Bc
        l = (lambda x, dt: x.astype(dt))(jnp.arange(L), A_re.dtype)
        P = jnp.exp(logdA[:, :, None] * l[None, None, :])
        K = jnp.einsum("dn,dnl,dn->dl", Cc, P, dB).real
        L2 = 2 * L
        Kp = jnp.pad(K, ((0, 0), (0, L)))
        up = (lambda x, *d: x.transpose(*d))(u, 0, 2, 1)
        up = jnp.pad(up, ((0, 0), (0, 0), (0, L)))
        Kf = (lambda x, axes=(-2,-1): jnp.fft.rfft2(x.astype(jnp.float32), axes=axes))(Kp[:, None, :], axes=(-2, -1))
        Uf = (lambda x, axes=(-2,-1): jnp.fft.rfft2(x.astype(jnp.float32), axes=axes))(up[:, :, None, :], axes=(-2, -1))
        Yf = Uf * Kf[None, :, :, :]
        y = (lambda x, s, axes=(-2,-1): jnp.fft.irfft2(x, s=s, axes=axes).astype(jnp.bfloat16))(Yf, (1, L2), axes=(-2, -1))[:, :, 0, :L]
        y = (lambda x, *d: x.transpose(*d))(y, 0, 2, 1) + u * Dskip[None, None, :]
        return y

    x = A_x
    x = x + _A_ref(_layernorm(x, axis=-1), A_wqkv, A_w_phi, A_wo)
    x = x + _B_ref(_layernorm(x, axis=-1), B_A_re, B_A_im, B_B_re, B_B_im, B_C_re, B_C_im, B_log_dt, B_Dskip)
    x = x + _A_ref(_layernorm(x, axis=-1), A_wqkv, A_w_phi, A_wo)
    x = x + _B_ref(_layernorm(x, axis=-1), B_A_re, B_A_im, B_B_re, B_B_im, B_C_re, B_C_im, B_log_dt, B_Dskip)
    return x
```

```python
import numpy as np
import jax
import jax.numpy as jnp
from jax import lax
import jax.experimental.pallas as pl
import jax.experimental.pallas.tpu as pltpu

F32 = jnp.float32
BF16 = jnp.bfloat16

S = 2048
D = 512
NT = 16
NS = 128
LOG2E = 1.4426950408889634

_R1 = [0, 0, 2, 4, 4, 4, 6, 8, 8, 8, 10, 12, 12, 12, 14, 16]
_R2 = [0, 0, 0, 4, 4, 4, 8, 8, 8, 8, 8, 12, 12, 12, 16, 16]
_R3 = [0, 0, 0, 0, 0, 8, 8, 8, 8, 8, 8, 8, 16, 16, 16, 16]
_HI = ([(0, r) for r in range(17)] + [(1, r) for r in (0, 4, 8, 12, 16)]
       + [(2, r) for r in (0, 8, 16)] + [(3, r) for r in (0, 8, 16)])
_HI_IDX = {qr: i for i, qr in enumerate(_HI)}
NHI = len(_HI)
NLO = 32


def _dft_table():
    n1 = np.arange(16, dtype=np.float64)[:, None, None]
    n2 = np.arange(128, dtype=np.float64)[None, :, None]
    k2 = np.arange(128, dtype=np.float64)[None, None, :]
    th = 2.0 * np.pi * (n1 + 16.0 * n2) * (k2 + 0.5) / 4096.0
    return np.concatenate([np.cos(th), -np.sin(th)], axis=2).astype(np.float32)


def _cmul(a, b):
    return (a[0] * b[0] - a[1] * b[1], a[0] * b[1] + a[1] * b[0])


def _csq(a):
    return (a[0] * a[0] - a[1] * a[1], (a[0] + a[0]) * a[1])


def _bfly4(x0, x1, x2, x3, sgn):
    a = (x0[0] + x2[0], x0[1] + x2[1])
    b = (x0[0] - x2[0], x0[1] - x2[1])
    c = (x1[0] + x3[0], x1[1] + x3[1])
    d = (x1[0] - x3[0], x1[1] - x3[1])
    y0 = (a[0] + c[0], a[1] + c[1])
    y2 = (a[0] - c[0], a[1] - c[1])
    if sgn < 0:
        y1 = (b[0] + d[1], b[1] - d[0])
        y3 = (b[0] - d[1], b[1] + d[0])
    else:
        y1 = (b[0] - d[1], b[1] + d[0])
        y3 = (b[0] + d[1], b[1] - d[0])
    return y0, y1, y2, y3


def _twiddle(x, m, sgn):
    m = m % 16
    if m == 0:
        return x
    if m == 4:
        return (x[1], -x[0]) if sgn < 0 else (-x[1], x[0])
    c = float(np.cos(2 * np.pi * m / 16))
    s = float(sgn * np.sin(2 * np.pi * m / 16))
    if m in (2, 6):
        h = float(np.sqrt(0.5))
        sc = 1.0 if c > 0 else -1.0
        ss = 1.0 if s > 0 else -1.0
        if sc * ss > 0:
            re = x[0] - x[1]
            im = x[0] + x[1]
            return (re * (h * sc), im * (h * sc))
        re = x[0] + x[1]
        im = x[1] - x[0]
        return (re * (h * sc), im * (h * sc))
    return (x[0] * c - x[1] * s, x[0] * s + x[1] * c)


def _fft16(x, sgn):
    t = [[None] * 4 for _ in range(4)]
    for b in range(4):
        y = _bfly4(x[b], x[4 + b], x[8 + b], x[12 + b], sgn)
        for c in range(4):
            t[b][c] = _twiddle(y[c], b * c, sgn)
    out = [None] * 16
    for c in range(4):
        y = _bfly4(t[0][c], t[1][c], t[2][c], t[3][c], sgn)
        for e in range(4):
            out[c + 4 * e] = y[e]
    return out


def _dot(a, b):
    return jnp.dot(a, b, preferred_element_type=F32)


def _dot_nt(a, b):
    return lax.dot_general(a, b, (((1,), (1,)), ((), ())), preferred_element_type=F32)


def _layernorm_t(xt):
    m = jnp.sum(xt, axis=0, keepdims=True) * (1.0 / D)
    xc = xt - m
    v = jnp.sum(xc * xc, axis=0, keepdims=True) * (1.0 / D)
    return xc * lax.rsqrt(v + 1e-5)


def _features(p):
    p3 = p.reshape(16, 8, 128)
    mx = jnp.max(p3, axis=0)
    mn = jnp.min(p3, axis=0)
    ep = jnp.exp2(p3 - mx[None])
    en = jnp.exp2(mn[None] - p3)
    rp = 1.0 / jnp.sum(ep, axis=0)
    rn = 1.0 / jnp.sum(en, axis=0)
    fp = (ep * rp[None]).reshape(128, 128)
    fn = (en * rn[None]).reshape(128, 128)
    return jnp.concatenate([fp, fn], axis=0).astype(BF16)


def _kernel(x_ref, wqkv_ref, wphi_ref, wo_ref, are_ref, aim_ref, bre_ref, bim_ref,
            cre_ref, cim_ref, ldt_ref, dsk_ref, mf_ref, out_ref,
            xs, X, Z, KF, PHQ, WALL, WOT, KVA, KVT, EH, EL, KS, DSK, P):
    lane128 = lax.broadcasted_iota(jnp.int32, (128, 128), 1)
    row128 = lax.broadcasted_iota(jnp.int32, (128, 128), 0)

    with jax.named_scope("wprep"):
        pm = jnp.where((row128 // 16 == lane128 % 8) & (row128 % 16 == lane128 // 8),
                       1.0, 0.0).astype(BF16)
        e16 = jnp.where(lax.broadcasted_iota(jnp.int32, (16, 128), 0)
                        == lax.broadcasted_iota(jnp.int32, (16, 128), 1) // 8,
                        1.0, 0.0).astype(BF16)
        hmask = (row128 // 16) == (lane128 % 8)
        for g in range(4):
            wp = wphi_ref[g * 128:(g + 1) * 128, :]
            bdt = jnp.where(hmask, _dot(wp, e16), 0.0).astype(BF16)
            for part in range(2):
                w = wqkv_ref[:, part * 512 + g * 128: part * 512 + (g + 1) * 128]
                t = _dot(w, bdt) * LOG2E
                WALL[part * 512 + g * 128: part * 512 + (g + 1) * 128, :] = t.T.astype(BF16)
            w = wqkv_ref[:, 1024 + g * 128: 1024 + (g + 1) * 128]
            WALL[1024 + g * 128: 1024 + (g + 1) * 128, :] = _dot(w, pm).T.astype(BF16)
            wot = wo_ref[g * 128:(g + 1) * 128, :].astype(F32).T.astype(BF16)
            WOT[:, g * 128:(g + 1) * 128] = _dot(wot, pm).astype(BF16)
        DSK[...] = jnp.broadcast_to(dsk_ref[...].astype(F32), (128, D)).T

    with jax.named_scope("kgen_e"):
        dtb = jnp.exp(ldt_ref[...].astype(F32)).astype(BF16).astype(F32)
        Z[0, :, 0:128] = jnp.broadcast_to(dtb, (128, D)).T

        RB = 16

        def ebody(i, carry):
            r0 = pl.multiple_of(i * RB, RB)
            rows = pl.ds(r0, RB)
            dt = Z[0, rows, 0:128]
            ar = dt * are_ref[rows, :].astype(F32)
            ai = dt * aim_ref[rows, :].astype(F32)
            db = (dt * bre_ref[rows, :].astype(F32), dt * bim_ref[rows, :].astype(F32))
            c0 = _cmul((cre_ref[rows, :].astype(F32), cim_ref[rows, :].astype(F32)), db)
            mag = jnp.exp(ar)
            w = {1: (mag * jnp.cos(ai), mag * jnp.sin(ai))}
            k = 1
            while k < 1024:
                w[2 * k] = _csq(w[k])
                k *= 2
            w[1536] = _cmul(w[1024], w[512])
            c = {0: c0}
            for b in (1, 2, 4, 8):
                for r in range(b):
                    c[r + b] = _cmul(c[r], w[b])
            c[16] = _cmul(c0, w[16])

            def put_hi(idx, v):
                rr = pl.ds(pl.multiple_of(idx * D + r0, RB), RB)
                EH[0, rr, :] = v[0]
                EH[1, rr, :] = -v[1]

            for idx, (q, r) in enumerate(_HI):
                put_hi(idx, c[r] if q == 0 else _cmul(c[r], w[512 * q]))
            dd = i // (128 // RB)
            g0 = r0 - dd * 128
            lo = {0: None}
            for b in (1, 2, 4, 8, 16):
                for j in range(b):
                    lo[j + b] = w[16 * b] if j == 0 else _cmul(lo[j], w[16 * b])
            for j in range(NLO):
                rr = pl.ds(pl.multiple_of((dd * NLO + j) * 128 + g0, RB), RB)
                if j == 0:
                    EL[0, rr, :] = jnp.ones((RB, 128), F32)
                    EL[1, rr, :] = jnp.zeros((RB, 128), F32)
                else:
                    EL[0, rr, :] = lo[j][0]
                    EL[1, rr, :] = lo[j][1]
            return carry

        lax.fori_loop(0, D // RB, ebody, 0)

    with jax.named_scope("kgen_mm"):
        def gbody(g, carry):
            a = jnp.concatenate([EH[c, pl.ds(g, NHI * 4, stride=128), :].astype(BF16)
                                 for c in range(2)], axis=1)
            b = jnp.concatenate([EL[c, pl.ds(g, NLO * 4, stride=128), :].astype(BF16)
                                 for c in range(2)], axis=1)
            KS[pl.ds(g, NHI * 4, stride=128), :] = _dot_nt(a, b)
            return carry

        lax.fori_loop(0, 128, gbody, 0, unroll=4)

    with jax.named_scope("kgen_asm"):
        for idx, (q, r) in enumerate(_HI):
            for dd in range(4):
                sh = ((q - dd) * 32) % 128
                if sh:
                    sl = slice((idx * 4 + dd) * 128, (idx * 4 + dd + 1) * 128)
                    KS[sl, :] = pltpu.roll(KS[sl, :], sh, 1)

        def slab(q, r, dd):
            i0 = (_HI_IDX[(q, r)] * 4 + dd) * 128
            return KS[i0:i0 + 128, :]

        for n1 in range(NT):
            parts = []
            for dd in range(4):
                t = jnp.where(lane128 < 96, slab(2, _R3[n1], dd), slab(3, _R3[n1], dd))
                t = jnp.where(lane128 < 64, slab(1, _R2[n1], dd), t)
                t = jnp.where(lane128 < 32, slab(0, _R1[n1], dd), t)
                t = jnp.where(lane128 < 16, slab(0, n1, dd), t)
                parts.append(t.astype(BF16))
            kt = jnp.concatenate(parts, axis=0)
            Z[n1] = _dot(kt, mf_ref[n1])

    with jax.named_scope("kgen_fft"):
        def kfbody(i, carry):
            rows = pl.ds(pl.multiple_of(i * 8, 8), 8)
            z = [(Z[j, rows, 0:128], Z[j, rows, 128:256]) for j in range(NT)]
            f = _fft16(z, -1)
            for j in range(NT):
                KF[j, rows, 0:128] = f[j][0] * (2.0 / 4096.0)
                KF[j, rows, 128:256] = f[j][1] * (2.0 / 4096.0)
            return carry

        lax.fori_loop(0, D // 8, kfbody, 0)

    ones16 = jnp.ones((16, 128), BF16)

    def a_pass1(n1, xt):
        xn = _layernorm_t(xt).astype(BF16)
        P[...] = _dot(WALL[...], xn)
        for g in range(4):
            PHQ[n1, g * 256:(g + 1) * 256, :] = _features(P[g * 128:(g + 1) * 128, :])
            fk = _features(P[512 + g * 128: 512 + (g + 1) * 128, :])
            va = jnp.concatenate(
                [P[1024 + g * 128: 1024 + (g + 1) * 128, :].astype(BF16), ones16], axis=0)
            KVA[g] += _dot_nt(va, fk)

    def a_mid():
        r = lax.broadcasted_iota(jnp.int32, (144, 256), 0)
        c = lax.broadcasted_iota(jnp.int32, (144, 256), 1)
        msk = (r % 8) == (c % 8)
        for g in range(4):
            KVT[g] = jnp.where(msk, KVA[g], 0.0).astype(BF16)

    def a_pass2_b_in(n1):
        os_ = []
        for g in range(4):
            rr = _dot(KVT[g], PHQ[n1, g * 256:(g + 1) * 256, :])
            rden = 1.0 / (rr[128:136, :] + 1e-6)
            o = rr[0:128, :].reshape(16, 8, 128) * rden[None]
            os_.append(o.reshape(128, 128).astype(BF16))
        o = jnp.concatenate(os_, axis=0)
        xt = X[n1] + _dot(WOT[...], o)
        u = _layernorm_t(xt).astype(BF16)
        X[n1] = xt + u.astype(F32) * DSK[...]
        Z[n1] = _dot(u, mf_ref[n1])

    def b_mid():
        def body(i, carry):
            rows = pl.ds(pl.multiple_of(i * 8, 8), 8)
            z = [(Z[j, rows, 0:128], Z[j, rows, 128:256]) for j in range(NT)]
            f = _fft16(z, -1)
            y = [_cmul(f[j], (KF[j, rows, 0:128], KF[j, rows, 128:256])) for j in range(NT)]
            v = _fft16(y, 1)
            for j in range(NT):
                Z[j, rows, 0:128] = v[j][0]
                Z[j, rows, 128:256] = v[j][1]
            return carry

        lax.fori_loop(0, D // 8, body, 0)

    def b_out(n1):
        return X[n1] + _dot_nt(Z[n1].astype(BF16), mf_ref[n1])

    for c in range(4):
        xs[c] = x_ref[:, c * 128:(c + 1) * 128].astype(F32)
    KVA[...] = jnp.zeros(KVA.shape, F32)

    with jax.named_scope("a1"):
        def l1(n1, carry):
            xt = jnp.concatenate([xs[c, pl.ds(n1, 128, stride=16), :].T for c in range(4)],
                                 axis=0)
            X[n1] = xt
            a_pass1(n1, xt)
            return carry
        lax.fori_loop(0, NT, l1, 0)
        a_mid()

    def l2(n1, carry):
        a_pass2_b_in(n1)
        return carry

    with jax.named_scope("a2"):
        lax.fori_loop(0, NT, l2, 0)
    with jax.named_scope("bmid"):
        b_mid()

    KVA[...] = jnp.zeros(KVA.shape, F32)
    with jax.named_scope("a1b"):
        def l3(n1, carry):
            xt = b_out(n1)
            X[n1] = xt
            a_pass1(n1, xt)
            return carry
        lax.fori_loop(0, NT, l3, 0)
        a_mid()
    with jax.named_scope("a2b"):
        lax.fori_loop(0, NT, l2, 0)
    with jax.named_scope("bmidb"):
        b_mid()
    with jax.named_scope("bout"):
        def l5(n1, carry):
            xt = b_out(n1)
            for c in range(4):
                xs[c, pl.ds(n1, 128, stride=16), :] = xt[c * 128:(c + 1) * 128, :].T
            return carry
        lax.fori_loop(0, NT, l5, 0)
        for c in range(4):
            out_ref[:, c * 128:(c + 1) * 128] = xs[c].astype(BF16)


@jax.jit
def pallas_interleave_layers__linear_kernel_hedgehog__ssm_conv_s4__prompt_kernel(
    A_x: jax.Array,
    A_wqkv: jax.Array,
    A_w_phi: jax.Array,
    A_wo: jax.Array,
    B_u: jax.Array,
    B_A_re: jax.Array,
    B_A_im: jax.Array,
    B_B_re: jax.Array,
    B_B_im: jax.Array,
    B_C_re: jax.Array,
    B_C_im: jax.Array,
    B_log_dt: jax.Array,
    B_Dskip: jax.Array,
):
    mf = jnp.asarray(_dft_table(), dtype=BF16)
    vm = pl.BlockSpec(memory_space=pltpu.VMEM)
    out = pl.pallas_call(
        _kernel,
        out_shape=jax.ShapeDtypeStruct((S, D), BF16),
        in_specs=[vm] * 13,
        out_specs=vm,
        scratch_shapes=[
            pltpu.VMEM((4, S, 128), F32),
            pltpu.VMEM((NT, D, 128), F32),
            pltpu.VMEM((NT, D, 256), F32),
            pltpu.VMEM((NT, D, 256), F32),
            pltpu.VMEM((NT, 1024, 128), BF16),
            pltpu.VMEM((1536, D), BF16),
            pltpu.VMEM((D, D), BF16),
            pltpu.VMEM((4, 144, 256), F32),
            pltpu.VMEM((4, 144, 256), BF16),
            pltpu.VMEM((2, NHI * D, 128), F32),
            pltpu.VMEM((2, NLO * D, 128), F32),
            pltpu.VMEM((NHI * D, 128), F32),
            pltpu.VMEM((D, 128), F32),
            pltpu.VMEM((1536, 128), F32),
        ],
        compiler_params=pltpu.CompilerParams(vmem_limit_bytes=110 * 1024 * 1024),
    )(A_x.reshape(S, D), A_wqkv, A_w_phi.reshape(D, 16), A_wo,
      B_A_re, B_A_im, B_B_re, B_B_im, B_C_re, B_C_im,
      B_log_dt.reshape(1, D), B_Dskip.reshape(1, D), mf)
    return out.reshape(1, S, D)
```

```python
import numpy as np
import jax
import jax.numpy as jnp
from jax import lax
import jax.experimental.pallas as pl
import jax.experimental.pallas.tpu as pltpu

F32 = jnp.float32
BF16 = jnp.bfloat16
U32 = jnp.uint32

S = 2048
D = 512
NT = 16
NS = 128
LOG2E = 1.4426950408889634

_R1 = [0, 0, 2, 4, 4, 4, 6, 8, 8, 8, 10, 12, 12, 12, 14, 16]
_R2 = [0, 0, 0, 4, 4, 4, 8, 8, 8, 8, 8, 12, 12, 12, 16, 16]
_R3 = [0, 0, 0, 0, 0, 8, 8, 8, 8, 8, 8, 8, 16, 16, 16, 16]
_HI = ([(0, r) for r in range(17)] + [(1, r) for r in (0, 4, 8, 12, 16)]
       + [(2, r) for r in (0, 8, 16)] + [(3, r) for r in (0, 8, 16)])
_HI_IDX = {qr: i for i, qr in enumerate(_HI)}
NHI = len(_HI)
NLO = 32
PITCH = 129


def _dft_table():
    n1 = np.arange(16, dtype=np.float64)[:, None, None]
    n2 = np.arange(128, dtype=np.float64)[None, :, None]
    k2 = np.arange(128, dtype=np.float64)[None, None, :]
    th = 2.0 * np.pi * (n1 + 16.0 * n2) * (k2 + 0.5) / 4096.0
    tab = np.concatenate([np.cos(th), -np.sin(th)], axis=2).astype(np.float32)
    bits = tab.astype(BF16).view(np.uint16).astype(np.uint32)
    return bits[:, 0::2, :] | (bits[:, 1::2, :] << 16)


def _cmul(a, b):
    return (a[0] * b[0] - a[1] * b[1], a[0] * b[1] + a[1] * b[0])


def _csq(a):
    return (a[0] * a[0] - a[1] * a[1], (a[0] + a[0]) * a[1])


def _bfly4(x0, x1, x2, x3, sgn):
    a = (x0[0] + x2[0], x0[1] + x2[1])
    b = (x0[0] - x2[0], x0[1] - x2[1])
    c = (x1[0] + x3[0], x1[1] + x3[1])
    d = (x1[0] - x3[0], x1[1] - x3[1])
    y0 = (a[0] + c[0], a[1] + c[1])
    y2 = (a[0] - c[0], a[1] - c[1])
    if sgn < 0:
        y1 = (b[0] + d[1], b[1] - d[0])
        y3 = (b[0] - d[1], b[1] + d[0])
    else:
        y1 = (b[0] - d[1], b[1] + d[0])
        y3 = (b[0] + d[1], b[1] - d[0])
    return y0, y1, y2, y3


def _twiddle(x, m, sgn):
    m = m % 16
    if m == 0:
        return x
    if m == 4:
        return (x[1], -x[0]) if sgn < 0 else (-x[1], x[0])
    c = float(np.cos(2 * np.pi * m / 16))
    s = float(sgn * np.sin(2 * np.pi * m / 16))
    if m in (2, 6):
        h = float(np.sqrt(0.5))
        sc = 1.0 if c > 0 else -1.0
        ss = 1.0 if s > 0 else -1.0
        if sc * ss > 0:
            re = x[0] - x[1]
            im = x[0] + x[1]
            return (re * (h * sc), im * (h * sc))
        re = x[0] + x[1]
        im = x[1] - x[0]
        return (re * (h * sc), im * (h * sc))
    return (x[0] * c - x[1] * s, x[0] * s + x[1] * c)


def _fft16(x, sgn):
    t = [[None] * 4 for _ in range(4)]
    for b in range(4):
        y = _bfly4(x[b], x[4 + b], x[8 + b], x[12 + b], sgn)
        for c in range(4):
            t[b][c] = _twiddle(y[c], b * c, sgn)
    out = [None] * 16
    for c in range(4):
        y = _bfly4(t[0][c], t[1][c], t[2][c], t[3][c], sgn)
        for e in range(4):
            out[c + 4 * e] = y[e]
    return out


def _fft8(x, sgn):
    a = [(x[n][0] + x[n + 4][0], x[n][1] + x[n + 4][1]) for n in range(4)]
    b = [_twiddle((x[n][0] - x[n + 4][0], x[n][1] - x[n + 4][1]), 2 * n, sgn) for n in range(4)]
    ya = _bfly4(a[0], a[1], a[2], a[3], sgn)
    yb = _bfly4(b[0], b[1], b[2], b[3], sgn)
    out = [None] * 8
    for m in range(4):
        out[2 * m] = ya[m]
        out[2 * m + 1] = yb[m]
    return out


def _dot(a, b):
    return jnp.dot(a, b, preferred_element_type=F32)


def _dot_nt(a, b):
    return lax.dot_general(a, b, (((1,), (1,)), ((), ())), preferred_element_type=F32)


def _layernorm_t(xt):
    m = jnp.sum(xt, axis=0, keepdims=True) * (1.0 / D)
    xc = xt - m
    v = jnp.sum(xc * xc, axis=0, keepdims=True) * (1.0 / D)
    return xc * lax.rsqrt(v + 1e-5)


def _pk(x):
    return pltpu.bitcast(x, U32)


def _up(w):
    return pltpu.bitcast(w, BF16)


def _pack2(a, b):
    return pltpu.pack_elementwise([a, b], packed_dtype=BF16)


def _unpack2(w, i):
    return pltpu.unpack_elementwise(w, index=i, packed_dtype=BF16, unpacked_dtype=F32)


def _features(p):
    p3 = p.reshape(8, 8, 128)
    mx = jnp.max(p3, axis=0)
    mx = jnp.maximum(mx, pltpu.roll(mx, 4, 0))
    mn = jnp.min(p3, axis=0)
    mn = jnp.minimum(mn, pltpu.roll(mn, 4, 0))
    ep = jnp.exp2(p3 - mx[None])
    en = jnp.exp2(mn[None] - p3)
    sp = jnp.sum(ep, axis=0)
    sn = jnp.sum(en, axis=0)
    rp = 1.0 / (sp + pltpu.roll(sp, 4, 0))
    rn = 1.0 / (sn + pltpu.roll(sn, 4, 0))
    return _pack2((ep * rp[None]).reshape(64, 128), (en * rn[None]).reshape(64, 128))


def _interleave(*stages):
    order = sorted(((k + 0.5) / n, i) for i, (_, n) in enumerate(stages) for k in range(n))
    for _, i in order:
        next(stages[i][0], None)
    for g, _ in stages:
        for _ in g:
            pass


def _colsum8(x):
    return jnp.sum(x.reshape(x.shape[0] // 8, 8, 128), axis=0)


def _ln_gen(first_pass, load, emit):
    s = None
    for c in range(4):
        t = _colsum8(first_pass(c))
        s = t if s is None else s + t
        yield
    m = jnp.sum(s, axis=0, keepdims=True) * (1.0 / D)
    v = None
    for c in range(4):
        xc = load(pl.ds(c * 128, 128)) - m
        t = _colsum8(xc * xc)
        v = t if v is None else v + t
        yield
    r = lax.rsqrt(jnp.sum(v, axis=0, keepdims=True) * (1.0 / D) + 1e-5)
    for c in range(4):
        xe = load(pl.ds(c * 128, 64, stride=2))
        xo = load(pl.ds(c * 128 + 1, 64, stride=2))
        emit(c, _pack2((xe - m) * r, (xo - m) * r), xe, xo)
        yield


LAG = 0
RBK = 64
NBK = D // RBK


def _kernel(x_hbm, wqkv_hbm, wphi_ref, wo_hbm, are_hbm, aim_hbm, bre_hbm, bim_hbm,
            cre_hbm, cim_hbm, ldt_ref, dsk_ref, mf_hbm, out_hbm,
            XP, WQ, WO, SSM, MF, XA, XB, KF, PHQ, WALL, WOT, KVA, KVT, EH, EL, KS, DSK, DT,
            XN0, XN1, FK0, FK1, VA0, VA1, O0, O1, XT0, XT1, U, ZA, ZS, VB0, VB1, sem):
    XN, FK, VA, O, XT = (XN0, XN1), (FK0, FK1), (VA0, VA1), (O0, O1), (XT0, XT1)
    VB = (VB0, VB1)
    ZS[0] = 0
    ZS[1] = 0
    lane128 = lax.broadcasted_iota(jnp.int32, (128, 128), 1)
    row128 = lax.broadcasted_iota(jnp.int32, (128, 128), 0)

    ssm_cp = [pltpu.make_async_copy(h, SSM.bitcast(BF16).at[k], sem.at[k])
              for k, h in enumerate((are_hbm, aim_hbm, bre_hbm, bim_hbm, cre_hbm, cim_hbm))]
    mf_cp = pltpu.make_async_copy(mf_hbm, MF, sem.at[6])
    wq_cp = pltpu.make_async_copy(wqkv_hbm, WQ.bitcast(BF16), sem.at[7])
    wo_cp = pltpu.make_async_copy(wo_hbm, WO.bitcast(BF16), sem.at[8])
    xpb = XP.bitcast(BF16)
    x_cp = [pltpu.make_async_copy(x_hbm.at[:, pl.ds(c * 128, 128)], xpb.at[c], sem.at[9 + c])
            for c in range(4)]
    for cp in ssm_cp + [mf_cp, wq_cp, wo_cp] + x_cp:
        cp.start()

    with jax.named_scope("kgen_e"):
        dtb = jnp.exp(ldt_ref[...].reshape(1, D).astype(F32)).astype(BF16).astype(F32)
        DT[...] = jnp.broadcast_to(dtb, (128, D)).T
        DSK[...] = jnp.broadcast_to(dsk_ref[...].reshape(1, D).astype(F32), (128, D)).T
        for cp in ssm_cp:
            cp.wait()

        RB = 16

        def ebody(i, carry):
            r0 = pl.multiple_of(i * RB, RB)
            rows = pl.ds(r0, RB)
            dt = DT[rows, :]
            hr = pl.ds(pl.multiple_of(i * (RB // 2), RB // 2), RB // 2)
            prm = [_up(SSM[k, hr, :]).astype(F32) for k in range(6)]
            ar = dt * prm[0]
            ai = dt * prm[1]
            db = (dt * prm[2], dt * prm[3])
            c0 = _cmul((prm[4], prm[5]), db)
            mag = jnp.exp(ar)
            w = {1: (mag * jnp.cos(ai), mag * jnp.sin(ai))}
            k = 1
            while k < 1024:
                w[2 * k] = _csq(w[k])
                k *= 2
            w[1536] = _cmul(w[1024], w[512])
            c = {0: c0}
            for b in (1, 2, 4, 8):
                for r in range(b):
                    c[r + b] = _cmul(c[r], w[b])
            c[16] = _cmul(c0, w[16])

            dd = i // (128 // RB)
            g0 = r0 - dd * 128

            def put_hi(idx, v):
                rr = pl.ds((idx * 4 + dd) * PITCH + 2 * g0, RB, stride=2)
                EH[0, rr, :] = v[0]
                EH[1, rr, :] = -v[1]

            for idx, (q, r) in enumerate(_HI):
                put_hi(idx, c[r] if q == 0 else _cmul(c[r], w[512 * q]))
            lo = {0: None}
            for b in (1, 2, 4, 8, 16):
                for j in range(b):
                    lo[j + b] = w[16 * b] if j == 0 else _cmul(lo[j], w[16 * b])
            for j in range(NLO):
                rr = pl.ds((dd * NLO + j) * PITCH + 2 * g0, RB, stride=2)
                if j == 0:
                    EL[0, rr, :] = jnp.ones((RB, 128), F32)
                    EL[1, rr, :] = jnp.zeros((RB, 128), F32)
                else:
                    EL[0, rr, :] = lo[j][0]
                    EL[1, rr, :] = lo[j][1]
            return carry

        lax.fori_loop(0, D // RB, ebody, 0)

    with jax.named_scope("kgen_mm"):
        def gbody(g, carry):
            acc = None
            for c in range(2):
                a = EH[c, pl.ds(2 * g, NHI * 4, stride=PITCH), :].astype(BF16)
                b = EL[c, pl.ds(2 * g, NLO * 4, stride=PITCH), :].astype(BF16)
                t = _dot_nt(a, b)
                acc = t if acc is None else acc + t
            KS[pl.ds(2 * g, NHI * 4, stride=PITCH), :] = acc
            return carry

        lax.fori_loop(0, 128, gbody, 0, unroll=4)

    with jax.named_scope("kgen_asm"):
        mf_cp.wait()
        for idx, (q, r) in enumerate(_HI):
            for dd in range(4):
                sh = ((q - dd) * 32) % 128
                if sh:
                    sl = pl.ds((idx * 4 + dd) * PITCH, 128, stride=2)
                    KS[sl, :] = pltpu.roll(KS[sl, :], sh, 1)

        def slab(q, r, dd):
            return KS[pl.ds((_HI_IDX[(q, r)] * 4 + dd) * PITCH, 128, stride=2), :]

        for n1 in range(NT):
            parts = []
            for dd in range(4):
                t = jnp.where(lane128 < 96, slab(2, _R3[n1], dd), slab(3, _R3[n1], dd))
                t = jnp.where(lane128 < 64, slab(1, _R2[n1], dd), t)
                t = jnp.where(lane128 < 32, slab(0, _R1[n1], dd), t)
                t = jnp.where(lane128 < 16, slab(0, n1, dd), t)
                parts.append(t.astype(BF16))
            kt = jnp.concatenate(parts, axis=0)
            KF[n1] = _dot(kt, _up(MF[n1]))

    with jax.named_scope("kgen_fft"):
        def kfbody(i, carry):
            rows = pl.ds(pl.multiple_of(i * 8, 8), 8)
            z = [(KF[j, rows, 0:128], KF[j, rows, 128:256]) for j in range(NT)]
            f = _fft16(z, -1)
            for j in range(NT):
                KF[j, rows, 0:128] = f[j][0] * (2.0 / 4096.0)
                KF[j, rows, 128:256] = f[j][1] * (2.0 / 4096.0)
            return carry

        lax.fori_loop(0, D // 8, kfbody, 0)

    with jax.named_scope("wprep"):
        wq_cp.wait()
        wo_cp.wait()
        hd = (lane128 // 64) * 4 + lane128 % 4
        fe = 2 * ((lane128 % 64) // 8) + (lane128 % 8) // 4
        hmask = (row128 // 16) == hd
        pm = jnp.where(hmask & (row128 % 16 == fe), 1.0, 0.0).astype(BF16)
        l16 = lax.broadcasted_iota(jnp.int32, (16, 128), 1)
        e16 = jnp.where(lax.broadcasted_iota(jnp.int32, (16, 128), 0)
                        == 2 * ((l16 % 64) // 8) + (l16 % 8) // 4, 1.0, 0.0).astype(BF16)
        k6 = lane128 % 64
        r6 = 32 * (k6 % 2) + k6 // 2
        a6 = 32 * (r6 % 2) + r6 // 2
        pmo = jnp.where(((row128 // 16) == (lane128 // 64) * 4 + a6 % 4)
                        & (row128 % 16 == 2 * (a6 // 8) + (a6 % 8) // 4), 1.0, 0.0).astype(BF16)
        wphi = wphi_ref[...].reshape(D, 16)
        wqu = WQ
        for g in range(4):
            wp = wphi[g * 128:(g + 1) * 128, :]
            bdt = jnp.where(hmask, _dot(wp, e16), 0.0).astype(BF16)
            for part in range(2):
                w = _up(wqu[:, part * 512 + g * 128: part * 512 + (g + 1) * 128])
                t = _dot(w, bdt) * LOG2E
                WALL[part * 256 + g * 64: part * 256 + (g + 1) * 64, :] = _pk(t.T.astype(BF16))
            w = _up(wqu[:, 1024 + g * 128: 1024 + (g + 1) * 128])
            WALL[512 + g * 64: 512 + (g + 1) * 64, :] = _pk(_dot(w, pm).T.astype(BF16))
            wot = _up(WO[g * 64:(g + 1) * 64, :]).astype(F32).T.astype(BF16)
            WOT[:, g * 128:(g + 1) * 128] = _pk(_dot(wot, pmo).astype(BF16))
        for b in range(2):
            VA[b][...] = jnp.full(VA[b].shape, 0x3F803F80, U32)
        XT1[...] = jnp.zeros(XT1.shape, F32)
        for cp in x_cp:
            cp.wait()

    xpu = XP

    def a1_s1(first, xsrc, i, par):
        def fp(c):
            if first:
                xt = _unpack2(xpu[c, pl.ds(i // 2, 128, stride=8), :].T, par)
                xsrc[i, c * 128:(c + 1) * 128, :] = xt
                return xt
            return xsrc[i, c * 128:(c + 1) * 128, :]

        def emit(c, w, xe, xo):
            XN[par][c * 64:(c + 1) * 64, :] = w

        return _ln_gen(fp, lambda rows: xsrc[i, rows, :], emit)

    def a1_s2(i, par):
        for c in range(4):
            p = _dot(_up(WALL[256 + c * 64: 256 + (c + 1) * 64, :]), _up(XN[par][...]))
            FK[par][c * 128:c * 128 + 64, :] = _features(p[0:64, :])
            FK[par][c * 128 + 64:(c + 1) * 128, :] = _features(p[64:128, :])
            yield
        for c in range(4):
            p = _dot(_up(WALL[512 + c * 64: 512 + (c + 1) * 64, :]), _up(XN[par][...]))
            VA[par][80 * c: 80 * c + 32, :] = _pack2(p[0:32, :], p[32:64, :])
            VA[par][80 * c + 40: 80 * c + 72, :] = _pack2(p[64:96, :], p[96:128, :])
            yield
        for c in range(4):
            p = _dot(_up(WALL[c * 64:(c + 1) * 64, :]), _up(XN[par][...]))
            PHQ[i, c * 128:c * 128 + 64, :] = _features(p[0:64, :])
            PHQ[i, c * 128 + 64:(c + 1) * 128, :] = _features(p[64:128, :])
            yield

    def a1_s3(par):
        for g in range(8):
            KVA[g] += _dot_nt(_up(VA[par][g * 40:(g + 1) * 40, :]),
                              _up(FK[par][g * 64:(g + 1) * 64, :]))
            yield

    def a_pass1(first, xsrc):
        KVA[...] = jnp.zeros(KVA.shape, F32)
        FK1[...] = jnp.zeros(FK1.shape, U32)
        _interleave((a1_s1(first, xsrc, 0, 0), 12))

        def body(jj, carry):
            i = 2 * jj
            _interleave((a1_s3(1), 8), (a1_s2(i, 0), 12), (a1_s1(first, xsrc, i + 1, 1), 12))
            _interleave((a1_s3(0), 8), (a1_s2(i + 1, 1), 12),
                        (a1_s1(first, xsrc, jnp.minimum(i + 2, NT - 2), 0), 12))
            return carry

        lax.fori_loop(0, NT // 2, body, 0)
        _interleave((a1_s3(1), 8))
        r = lax.broadcasted_iota(jnp.int32, (40, 128), 0)
        c = lax.broadcasted_iota(jnp.int32, (40, 128), 1)
        msk = (r % 4) == ((c // 2) % 4)
        for g in range(8):
            KVT[g] = _pack2(jnp.where(msk, KVA[g, pl.ds(0, 40, stride=2), :], 0.0),
                            jnp.where(msk, KVA[g, pl.ds(1, 40, stride=2), :], 0.0))

    def a2_s1(i, par):
        for g in range(8):
            rr = _dot(_up(KVT[g]), _up(PHQ[i, g * 64:(g + 1) * 64, :]))
            rden = 1.0 / (rr[64:72, :] + 1e-6)
            o = (rr[0:64, :].reshape(8, 8, 128) * rden[None]).reshape(64, 128)
            O[par][g * 32:(g + 1) * 32, :] = _pack2(o[0:32, :], o[32:64, :])
            yield

    def a2_s2(xsrc, i, par):
        for c in range(4):
            XT[par][c * 128:(c + 1) * 128, :] = (
                xsrc[i, c * 128:(c + 1) * 128, :]
                + _dot(_up(WOT[c * 64:(c + 1) * 64, :]), _up(O[par][...])))
            yield

    def a2_s3(xdst, i, par):
        def emit(c, w, xe, xo):
            U[i, c * 64:(c + 1) * 64, :] = w
            re = pl.ds(c * 128, 64, stride=2)
            ro = pl.ds(c * 128 + 1, 64, stride=2)
            xdst[i, re, :] = xe + _unpack2(w, 0) * DSK[re, :]
            xdst[i, ro, :] = xo + _unpack2(w, 1) * DSK[ro, :]

        return _ln_gen(lambda c: XT[par][c * 128:(c + 1) * 128, :],
                       lambda rows: XT[par][rows, :], emit)

    def a_pass2(xsrc, xdst):
        _interleave((a2_s1(0, 0), 8))

        def body(jj, carry):
            i = 2 * jj
            _interleave((a2_s3(xdst, jnp.where(jj == 0, NT, i - 1), 1), 12),
                        (a2_s2(xsrc, i, 0), 4), (a2_s1(i + 1, 1), 8))
            _interleave((a2_s3(xdst, i, 0), 12), (a2_s2(xsrc, i + 1, 1), 4),
                        (a2_s1(jnp.minimum(i + 2, NT - 1), 0), 8))
            return carry

        lax.fori_loop(0, NT // 2, body, 0)
        _interleave((a2_s3(xdst, NT - 1, 1), 12))

    def b_f(j, par):
        rows = pl.ds(pl.multiple_of(j * (RBK // 2), RBK // 2), RBK // 2)
        pz = ZS[0] + par
        for n in range(8):
            z0 = _dot(_up(U[n, rows, :]), _up(MF[n]))
            z1 = _dot(_up(U[n + 8, rows, :]), _up(MF[n + 8]))
            ZA[pz, n] = z0 + z1
            ZA[pz, n + 8] = z0 - z1
            yield

    def b_m(j, par):
        pz = ZS[1] + par
        for s in range(RBK // 8):
            rr = pl.ds(s * 8, 8)
            kr = pl.ds(pl.multiple_of(j * RBK + s * 8, 8), 8)
            for h in range(2):
                z = [(ZA[pz, 8 * h + n, rr, 0:128], ZA[pz, 8 * h + n, rr, 128:256])
                     for n in range(8)]
                if h:
                    z = [_twiddle(z[n], n, -1) for n in range(8)]
                f = _fft8(z, -1)
                y = [_cmul(f[m], (KF[2 * m + h, kr, 0:128], KF[2 * m + h, kr, 128:256]))
                     for m in range(8)]
                v = _fft8(y, 1)
                if h:
                    v = [_twiddle(v[n], n, 1) for n in range(8)]
                for n in range(8):
                    VB[par][2 * (8 * h + n), rr, :] = v[n][0]
                    VB[par][2 * (8 * h + n) + 1, rr, :] = v[n][1]
                yield

    def b_i(xb, j, vsrc):
        rs = pl.ds(pl.multiple_of(j * RBK, RBK), RBK)
        ev = pl.ds(0, RBK // 2, stride=2)
        od = pl.ds(1, RBK // 2, stride=2)
        pz = ZS[0] + 2
        for n in range(8):
            v0, v1 = [], []
            for c in range(2):
                ee, eo = vsrc[2 * n + c, ev, :], vsrc[2 * n + c, od, :]
                oe, oo = vsrc[2 * n + 16 + c, ev, :], vsrc[2 * n + 16 + c, od, :]
                v0.append(_pack2(ee + oe, eo + oo))
                v1.append(_pack2(ee - oe, eo - oo))
            xb[n, rs, :] += _dot_nt(_up(jnp.concatenate(v0, axis=1)), _up(MF[n]))
            t = xb[n + 8, rs, :] + _dot_nt(_up(jnp.concatenate(v1, axis=1)), _up(MF[n + 8]))
            xb[n + 8, rs, :] = t
            ZA[pz, 0, 0:8, 0:128] = t[RBK - 8:RBK, :]
            yield

    def b_step(gi, gm, gf):
        for k in range(LAG):
            next(gm)
        for k in range(8):
            next(gm, None)
            next(gf)
            next(gm, None)
            next(gi)

    def b_phase(xb, first):
        _interleave((b_f(0, 0), 8))
        VB1[...] = jnp.zeros(VB1.shape, F32)

        def body(jj, carry):
            j = 2 * jj + 1
            b_step(b_i(xb, jnp.maximum(j - 2, 0), VB[1]), b_m(j - 1, 0), b_f(j, 1))

            @pl.when(jj >= 0)
            def _():
                b_step(b_i(xb, j - 1, VB[0]), b_m(j, 1), b_f(jnp.minimum(j + 1, NBK - 1), 0))
            return carry

        lax.fori_loop(0, NBK // 2, body, 0)
        _interleave((b_i(xb, NBK - 1, VB[1]), 8))

    with jax.named_scope("a1"):
        a_pass1(True, XA)
    with jax.named_scope("a2"):
        a_pass2(XA, XB)
    with jax.named_scope("b"):
        b_phase(XB, True)
    with jax.named_scope("a1b"):
        a_pass1(False, XB)
    with jax.named_scope("a2b"):
        a_pass2(XB, XA)
    with jax.named_scope("bb"):
        b_phase(XA, False)
    with jax.named_scope("out"):
        o_cp = [pltpu.make_async_copy(xpb.at[c], out_hbm.at[:, pl.ds(c * 128, 128)], sem.at[c])
                for c in range(4)]
        for c in range(4):
            for m in range(8):
                w = pltpu.pack_elementwise(
                    [XA[2 * m, c * 128:(c + 1) * 128, :], XA[2 * m + 1, c * 128:(c + 1) * 128, :]],
                    packed_dtype=BF16)
                xpu[c, pl.ds(m, 128, stride=8), :] = w.T
            o_cp[c].start()
        for cp in o_cp:
            cp.wait()


@jax.jit
def pallas_interleave_layers__linear_kernel_hedgehog__ssm_conv_s4__prompt_kernel(
    A_x: jax.Array,
    A_wqkv: jax.Array,
    A_w_phi: jax.Array,
    A_wo: jax.Array,
    B_u: jax.Array,
    B_A_re: jax.Array,
    B_A_im: jax.Array,
    B_B_re: jax.Array,
    B_B_im: jax.Array,
    B_C_re: jax.Array,
    B_C_im: jax.Array,
    B_log_dt: jax.Array,
    B_Dskip: jax.Array,
):
    mf = jnp.asarray(_dft_table())
    vm = pl.BlockSpec(memory_space=pltpu.VMEM)
    hb = pl.BlockSpec(memory_space=pl.ANY)
    out = pl.pallas_call(
        _kernel,
        out_shape=jax.ShapeDtypeStruct((S, D), BF16),
        in_specs=[hb, hb, vm, hb, hb, hb, hb, hb, hb, hb, vm, vm, hb],
        out_specs=hb,
        scratch_shapes=[
            pltpu.VMEM((4, S // 2, 128), U32),
            pltpu.VMEM((D // 2, 3 * D), U32),
            pltpu.VMEM((D // 2, D), U32),
            pltpu.VMEM((6, D // 2, NS), U32),
            pltpu.VMEM((NT, 64, 256), U32),
            pltpu.VMEM((NT + 1, D + RBK, 128), F32),
            pltpu.VMEM((NT + 1, D + RBK, 128), F32),
            pltpu.VMEM((NT, D, 256), F32),
            pltpu.VMEM((NT, 512, 128), U32),
            pltpu.VMEM((768, D), U32),
            pltpu.VMEM((256, D), U32),
            pltpu.VMEM((8, 80, 128), F32),
            pltpu.VMEM((8, 40, 128), U32),
            pltpu.VMEM((2, NHI * 4 * PITCH + 136, 128), F32),
            pltpu.VMEM((2, NLO * 4 * PITCH + 128, 128), F32),
            pltpu.VMEM((NHI * 4 * PITCH + 136, 128), F32),
            pltpu.VMEM((D, 128), F32),
            pltpu.VMEM((D, 128), F32),
            pltpu.VMEM((256, 128), U32),
            pltpu.VMEM((256, 128), U32),
            pltpu.VMEM((512, 128), U32),
            pltpu.VMEM((512, 128), U32),
            pltpu.VMEM((320, 128), U32),
            pltpu.VMEM((320, 128), U32),
            pltpu.VMEM((256, 128), U32),
            pltpu.VMEM((256, 128), U32),
            pltpu.VMEM((D, 128), F32),
            pltpu.VMEM((D, 128), F32),
            pltpu.VMEM((NT + 1, 256, 128), U32),
            pltpu.VMEM((3, NT, RBK, 256), F32),
            pltpu.SMEM((2,), jnp.int32),
            pltpu.VMEM((2 * NT, RBK, 128), F32),
            pltpu.VMEM((2 * NT, RBK, 128), F32),
            pltpu.SemaphoreType.DMA((13,)),
        ],
        compiler_params=pltpu.CompilerParams(vmem_limit_bytes=110 * 1024 * 1024),
    )(A_x.reshape(S, D), A_wqkv, A_w_phi, A_wo,
      B_A_re, B_A_im, B_B_re, B_B_im, B_C_re, B_C_im,
      B_log_dt, B_Dskip, mf)
    return out.reshape(1, S, D)
```

```python
import numpy as np
import jax
import jax.numpy as jnp
from jax import lax
import jax.experimental.pallas as pl
import jax.experimental.pallas.tpu as pltpu

F32 = jnp.float32
BF16 = jnp.bfloat16
U32 = jnp.uint32

S = 2048
D = 512
NT = 16
NS = 128
LOG2E = 1.4426950408889634

_R1 = [0, 0, 2, 4, 4, 4, 6, 8, 8, 8, 10, 12, 12, 12, 14, 16]
_R2 = [0, 0, 0, 4, 4, 4, 8, 8, 8, 8, 8, 12, 12, 12, 16, 16]
_R3 = [0, 0, 0, 0, 0, 8, 8, 8, 8, 8, 8, 8, 16, 16, 16, 16]
_HI = ([(0, r) for r in range(17)] + [(1, r) for r in (0, 4, 8, 12, 16)]
       + [(2, r) for r in (0, 8, 16)] + [(3, r) for r in (0, 8, 16)])
_HI_IDX = {qr: i for i, qr in enumerate(_HI)}
NHI = len(_HI)
NLO = 32
GB = 16
EP = 2 * GB + 1
PITCH = 129


def _dft_table():
    n1 = np.arange(16, dtype=np.float64)[:, None, None]
    n2 = np.arange(128, dtype=np.float64)[None, :, None]
    k2 = np.arange(128, dtype=np.float64)[None, None, :]
    th = 2.0 * np.pi * (n1 + 16.0 * n2) * (k2 + 0.5) / 4096.0
    tab = np.concatenate([np.cos(th), -np.sin(th)], axis=2).astype(np.float32)
    bits = tab.astype(BF16).view(np.uint16).astype(np.uint32)
    return bits[:, 0::2, :] | (bits[:, 1::2, :] << 16)


def _cmul(a, b):
    return (a[0] * b[0] - a[1] * b[1], a[0] * b[1] + a[1] * b[0])


def _csq(a):
    return (a[0] * a[0] - a[1] * a[1], (a[0] + a[0]) * a[1])


def _sincos(x):
    big = 12582912.0
    kf = x * 0.6366197723675814 + big
    ki = pltpu.bitcast(kf, jnp.int32)
    k = kf - big
    r = x - k * 1.5703125
    r = r - k * 4.837512969970703125e-4
    r = r - k * 7.54978995489188216e-8
    r = jnp.minimum(jnp.maximum(r, -1.0), 1.0)
    z = r * r
    ps = ((-1.9515295891e-4 * z + 8.3321608736e-3) * z - 1.6666654611e-1) * z * r + r
    pc = (((2.443315711809948e-5 * z - 1.388731625493765e-3) * z + 4.166664568298827e-2) * z
          - 0.5) * z + 1.0
    odd = (ki & 1) == 1
    sn = jnp.where(odd, pc, ps)
    cs = jnp.where(odd, ps, pc)
    sgs = (ki & 2) << 30
    sgc = ((ki + 1) & 2) << 30
    sn = pltpu.bitcast(pltpu.bitcast(sn, jnp.int32) ^ sgs, F32)
    cs = pltpu.bitcast(pltpu.bitcast(cs, jnp.int32) ^ sgc, F32)
    return sn, cs


def _bfly4(x0, x1, x2, x3, sgn):
    a = (x0[0] + x2[0], x0[1] + x2[1])
    b = (x0[0] - x2[0], x0[1] - x2[1])
    c = (x1[0] + x3[0], x1[1] + x3[1])
    d = (x1[0] - x3[0], x1[1] - x3[1])
    y0 = (a[0] + c[0], a[1] + c[1])
    y2 = (a[0] - c[0], a[1] - c[1])
    if sgn < 0:
        y1 = (b[0] + d[1], b[1] - d[0])
        y3 = (b[0] - d[1], b[1] + d[0])
    else:
        y1 = (b[0] - d[1], b[1] + d[0])
        y3 = (b[0] + d[1], b[1] - d[0])
    return y0, y1, y2, y3


def _twiddle(x, m, sgn):
    m = m % 16
    if m == 0:
        return x
    if m == 4:
        return (x[1], -x[0]) if sgn < 0 else (-x[1], x[0])
    c = float(np.cos(2 * np.pi * m / 16))
    s = float(sgn * np.sin(2 * np.pi * m / 16))
    if m in (2, 6):
        h = float(np.sqrt(0.5))
        sc = 1.0 if c > 0 else -1.0
        ss = 1.0 if s > 0 else -1.0
        if sc * ss > 0:
            re = x[0] - x[1]
            im = x[0] + x[1]
            return (re * (h * sc), im * (h * sc))
        re = x[0] + x[1]
        im = x[1] - x[0]
        return (re * (h * sc), im * (h * sc))
    return (x[0] * c - x[1] * s, x[0] * s + x[1] * c)


def _fft16(x, sgn):
    t = [[None] * 4 for _ in range(4)]
    for b in range(4):
        y = _bfly4(x[b], x[4 + b], x[8 + b], x[12 + b], sgn)
        for c in range(4):
            t[b][c] = _twiddle(y[c], b * c, sgn)
    out = [None] * 16
    for c in range(4):
        y = _bfly4(t[0][c], t[1][c], t[2][c], t[3][c], sgn)
        for e in range(4):
            out[c + 4 * e] = y[e]
    return out


def _fft8(x, sgn):
    a = [(x[n][0] + x[n + 4][0], x[n][1] + x[n + 4][1]) for n in range(4)]
    b = [_twiddle((x[n][0] - x[n + 4][0], x[n][1] - x[n + 4][1]), 2 * n, sgn) for n in range(4)]
    ya = _bfly4(a[0], a[1], a[2], a[3], sgn)
    yb = _bfly4(b[0], b[1], b[2], b[3], sgn)
    out = [None] * 8
    for m in range(4):
        out[2 * m] = ya[m]
        out[2 * m + 1] = yb[m]
    return out


def _dot(a, b):
    return jnp.dot(a, b, preferred_element_type=F32)


def _dot_nt(a, b):
    return lax.dot_general(a, b, (((1,), (1,)), ((), ())), preferred_element_type=F32)


def _layernorm_t(xt):
    m = jnp.sum(xt, axis=0, keepdims=True) * (1.0 / D)
    xc = xt - m
    v = jnp.sum(xc * xc, axis=0, keepdims=True) * (1.0 / D)
    return xc * lax.rsqrt(v + 1e-5)


def _pk(x):
    return pltpu.bitcast(x, U32)


def _up(w):
    return pltpu.bitcast(w, BF16)


def _pack2(a, b):
    return pltpu.pack_elementwise([a, b], packed_dtype=BF16)


def _unpack2(w, i):
    return pltpu.unpack_elementwise(w, index=i, packed_dtype=BF16, unpacked_dtype=F32)


def _features(p):
    p3 = p.reshape(8, 8, 128)
    mx = jnp.max(p3, axis=0)
    mx = jnp.maximum(mx, pltpu.roll(mx, 4, 0))
    mn = jnp.min(p3, axis=0)
    mn = jnp.minimum(mn, pltpu.roll(mn, 4, 0))
    ep = jnp.exp2(p3 - mx[None])
    en = jnp.exp2(mn[None] - p3)
    sp = jnp.sum(ep, axis=0)
    sn = jnp.sum(en, axis=0)
    rp = 1.0 / (sp + pltpu.roll(sp, 4, 0))
    rn = 1.0 / (sn + pltpu.roll(sn, 4, 0))
    return _pack2((ep * rp[None]).reshape(64, 128), (en * rn[None]).reshape(64, 128))


def _interleave(*stages):
    order = []
    for i, st in enumerate(stages):
        lo, hi = st[2:] if len(st) > 2 else (0.0, 1.0)
        order += [(lo + (hi - lo) * (k + 0.5) / st[1], i) for k in range(st[1])]
    for _, i in sorted(order):
        next(stages[i][0], None)
    for st in stages:
        for _ in st[0]:
            pass


def _colsum8(x):
    return jnp.sum(x.reshape(x.shape[0] // 8, 8, 128), axis=0)


def _ln_gen(first_pass, load, emit):
    s = None
    for c in range(4):
        t = _colsum8(first_pass(c))
        s = t if s is None else s + t
        yield
    m = jnp.sum(s, axis=0, keepdims=True) * (1.0 / D)
    v = None
    for c in range(4):
        xc = load(pl.ds(c * 128, 128)) - m
        t = _colsum8(xc * xc)
        v = t if v is None else v + t
        yield
    r = lax.rsqrt(jnp.sum(v, axis=0, keepdims=True) * (1.0 / D) + 1e-5)
    for c in range(4):
        xe = load(pl.ds(c * 128, 64, stride=2))
        xo = load(pl.ds(c * 128 + 1, 64, stride=2))
        emit(c, _pack2((xe - m) * r, (xo - m) * r), xe, xo)
        yield


LAG = 0
RBK = 64
NBK = D // RBK


def _kernel(x_hbm, wqkv_hbm, wphi_ref, wo_hbm, are_hbm, aim_hbm, bre_hbm, bim_hbm,
            cre_hbm, cim_hbm, ldt_ref, dsk_ref, mf_hbm, out_hbm,
            XP, WQ, WO, SSM, MF, XA, XB, KF, PHQ, WALL, WOT, KVA, KVT, EH0, EH1, EL0, EL1, EW, KS, DSK, DT,
            U, ZA, ZS, VB0, VB1, sem, *bufs):
    XN, FK, VA, O, XT = [bufs[4 * k:4 * k + 4] for k in range(5)]
    VB = (VB0, VB1)
    EHS, ELS = (EH0, EH1), (EL0, EL1)
    ZS[0] = 0
    ZS[1] = 0
    lane128 = lax.broadcasted_iota(jnp.int32, (128, 128), 1)
    row128 = lax.broadcasted_iota(jnp.int32, (128, 128), 0)

    ssm_cp = [pltpu.make_async_copy(h, SSM.bitcast(BF16).at[k], sem.at[k])
              for k, h in enumerate((are_hbm, aim_hbm, bre_hbm, bim_hbm, cre_hbm, cim_hbm))]
    mf_cp = pltpu.make_async_copy(mf_hbm, MF, sem.at[6])
    wq_cp = pltpu.make_async_copy(wqkv_hbm, WQ.bitcast(BF16), sem.at[7])
    wo_cp = pltpu.make_async_copy(wo_hbm, WO.bitcast(BF16), sem.at[8])
    xpb = XP.bitcast(BF16)
    x_cp = [pltpu.make_async_copy(x_hbm.at[:, pl.ds(c * 128, 128)], xpb.at[c], sem.at[9 + c])
            for c in range(4)]
    for cp in ssm_cp + [mf_cp, wq_cp, wo_cp] + x_cp:
        cp.start()

    with jax.named_scope("kgen_e"):
        dtb = jnp.exp(ldt_ref[...].reshape(1, D).astype(F32)).astype(BF16).astype(F32)
        DT[...] = jnp.broadcast_to(dtb, (128, D)).T
        DSK[...] = jnp.broadcast_to(dsk_ref[...].reshape(1, D).astype(F32), (128, D)).T
        for cp in ssm_cp:
            cp.wait()


    with jax.named_scope("kgen_e1"):
        def e1body(i, carry):
            hr = pl.ds(pl.multiple_of(i * 16, 16), 16)
            raw = [SSM[k, hr, :] for k in range(6)]
            for par in range(2):
                dt = DT[pl.ds(i * 32 + par, 16, stride=2), :]
                prm = [_unpack2(raw[k], par) for k in range(6)]
                dts = dt * (2.0 / 4096.0)
                c0 = _cmul((prm[4], prm[5]), (dts * prm[2], dts * prm[3]))
                mag = jnp.exp(dt * prm[0])
                sn, cs = _sincos(dt * prm[1])
                for k, v in enumerate((mag * cs, mag * sn, c0[0], c0[1])):
                    for h in range(2):
                        EW[k, pl.ds(pl.multiple_of(i * 32 + 16 * h + 8 * par, 8), 8), :] = (
                            v[8 * h:8 * h + 8, :])
            return carry

        lax.fori_loop(0, D // 32, e1body, 0)

    def e_piece(blk, dd, hf, par):
        rows = pl.ds(pl.multiple_of(dd * 128 + blk * GB + 8 * hf, 8), 8)
        EH, EL = EHS[par], ELS[par]
        w = {1: (EW[0, rows, :], EW[1, rows, :])}
        c = {0: (EW[2, rows, :], EW[3, rows, :])}

        def put(ref, n, k, u, v):
            rr = pl.ds((dd * n + k) * EP + 16 * hf, 8, stride=2)
            for cc in range(2):
                ref[cc, rr, :] = _pack2(u[cc], v[cc])

        for b in (1, 2, 4, 8):
            w[2 * b] = _csq(w[b])
            for r in range(b):
                c[r + b] = _cmul(c[r], w[b])
            if b == 1:
                put(EH, NHI // 2, 0, c[0], c[1])
            else:
                for r in range(b, 2 * b, 2):
                    put(EH, NHI // 2, r // 2, c[r], c[r + 1])
            if b >= 4:
                yield
        c[16] = _cmul(c[0], w[16])
        lo = {0: (jnp.ones((8, 128), F32), jnp.zeros((8, 128), F32))}
        for b in (1, 2, 4, 8, 16):
            w[32 * b] = _csq(w[16 * b])
            for j in range(b):
                lo[j + b] = w[16 * b] if j == 0 else _cmul(lo[j], w[16 * b])
                if b == 1:
                    put(EL, NLO // 2, 0, lo[0], lo[1])
                elif j % 2:
                    put(EL, NLO // 2, (j + b) // 2, lo[j + b - 1], lo[j + b])
                if b == 16 and j == 7:
                    yield
            if b >= 4:
                yield
        w[1024] = _csq(w[512])
        w[1536] = _cmul(w[1024], w[512])
        hi = [c[r] if q == 0 else _cmul(c[r], w[512 * q]) for q, r in _HI[16:]]
        for k in range(6):
            put(EH, NHI // 2, 8 + k, hi[2 * k], hi[2 * k + 1])
        yield

    def e_blk(blk, par):
        for hf in range(GB // 8):
            for dd in range(4):
                yield from e_piece(blk, dd, hf, par)

    def mm_blk(blk, par):
        for g in range(GB):
            t = [_dot_nt(_up(EHS[par][c, pl.ds(2 * g, NHI * 2, stride=EP), :]),
                         _up(ELS[par][c, pl.ds(2 * g, NLO * 2, stride=EP), :])) for c in range(2)]
            KS[pl.ds(2 * GB * blk + 2 * g, NHI * 4, stride=PITCH), :] = t[0] - t[1]
            yield

    with jax.named_scope("kgen_e2"):
        _interleave((e_blk(0, 0), 28))

        def ebody(jj, carry):
            @pl.when(jj >= -1)
            def _():
                _interleave((mm_blk(2 * jj, 0), GB), (e_blk(2 * jj + 1, 1), 28 * GB // 8))

            @pl.when(jj >= 0)
            def _():
                _interleave((mm_blk(2 * jj + 1, 1), GB),
                            (e_blk(jnp.minimum(2 * jj + 2, 128 // GB - 1), 0), 28 * GB // 8))
            return carry

        lax.fori_loop(0, 64 // GB, ebody, 0)

    with jax.named_scope("kgen_asm"):
        mf_cp.wait()
        for idx, (q, r) in enumerate(_HI):
            for dd in range(4):
                sh = ((q - dd) * 32) % 128
                if sh:
                    sl = pl.ds((dd * NHI + idx) * PITCH, 128, stride=2)
                    KS[sl, :] = pltpu.roll(KS[sl, :], sh, 1)

        def slab(q, r, dd):
            return KS[pl.ds((dd * NHI + _HI_IDX[(q, r)]) * PITCH, 128, stride=2), :]

        for n1 in range(NT):
            parts = []
            for dd in range(4):
                t = jnp.where(lane128 < 96, slab(2, _R3[n1], dd), slab(3, _R3[n1], dd))
                t = jnp.where(lane128 < 64, slab(1, _R2[n1], dd), t)
                t = jnp.where(lane128 < 32, slab(0, _R1[n1], dd), t)
                t = jnp.where(lane128 < 16, slab(0, n1, dd), t)
                t = t.reshape(8, 16, 128)
                parts.append(_pack2(t[:, 0:8, :], t[:, 8:16, :]).reshape(64, 128))
            kt = jnp.concatenate(parts, axis=0)
            KF[n1] = _dot(_up(kt), _up(MF[n1]))

    def kfft(p0, n):
        for k in range(n):
            rows = pl.ds(pl.multiple_of((p0 + k) * 8, 8), 8)
            z = [(KF[j, rows, 0:128], KF[j, rows, 128:256]) for j in range(NT)]
            f = _fft16(z, -1)
            for j in range(NT):
                KF[j, rows, 0:128] = f[j][0]
                KF[j, rows, 128:256] = f[j][1]
            yield

    with jax.named_scope("wprep"):
        wq_cp.wait()
        wo_cp.wait()
        hd = (lane128 // 64) * 4 + lane128 % 4
        fe = 2 * ((lane128 % 64) // 8) + (lane128 % 8) // 4
        hmask = (row128 // 16) == hd
        pm = jnp.where(hmask & (row128 % 16 == fe), 1.0, 0.0).astype(BF16)
        l16 = lax.broadcasted_iota(jnp.int32, (16, 128), 1)
        e16 = jnp.where(lax.broadcasted_iota(jnp.int32, (16, 128), 0)
                        == 2 * ((l16 % 64) // 8) + (l16 % 8) // 4, 1.0, 0.0).astype(BF16)
        k6 = lane128 % 64
        r6 = 32 * (k6 % 2) + k6 // 2
        a6 = 32 * (r6 % 2) + r6 // 2
        pmo = jnp.where(((row128 // 16) == (lane128 // 64) * 4 + a6 % 4)
                        & (row128 % 16 == 2 * (a6 // 8) + (a6 % 8) // 4), 1.0, 0.0).astype(BF16)
        wphi = wphi_ref[...].reshape(D, 16)
        wqu = WQ
        for g in range(4):
            wp = wphi[g * 128:(g + 1) * 128, :]
            bdt = jnp.where(hmask, _dot(wp, e16), 0.0).astype(BF16)
            for part in range(2):
                w = _up(wqu[:, part * 512 + g * 128: part * 512 + (g + 1) * 128])
                t = _dot(w, bdt) * LOG2E
                WALL[part * 256 + g * 64: part * 256 + (g + 1) * 64, :] = _pk(t.T.astype(BF16))
            w = _up(wqu[:, 1024 + g * 128: 1024 + (g + 1) * 128])
            WALL[512 + g * 64: 512 + (g + 1) * 64, :] = _pk(_dot(w, pm).T.astype(BF16))
            wot = _up(WO[g * 64:(g + 1) * 64, :]).astype(F32).T.astype(BF16)
            WOT[:, g * 128:(g + 1) * 128] = _pk(_dot(wot, pmo).astype(BF16))
        for b in range(4):
            VA[b][...] = jnp.full(VA[b].shape, 0x3F803F80, U32)
        for cp in x_cp:
            cp.wait()

    xpu = XP

    def _chain(*gens):
        for g in gens:
            yield from g

    def a1_s0(xsrc, i, sl):
        for c in range(4):
            w = xpu[c, pl.ds(i // 2, 128, stride=8), :].T
            for par in range(2):
                XT[sl + par][c * 128:(c + 1) * 128, :] = _unpack2(w, par)
            yield

    def a1_s1(first, xsrc, i, sl):
        def emit(c, w, xe, xo):
            XN[sl][c * 64:(c + 1) * 64, :] = w

        load = (lambda rows: XT[sl][rows, :]) if first else (lambda rows: xsrc[i, rows, :])

        def fp(c):
            xt = load(pl.ds(c * 128, 128))
            if first:
                xsrc[i, c * 128:(c + 1) * 128, :] = xt
            return xt

        return _ln_gen(fp, load, emit)

    def a1_s2(i, sl):
        for c in range(4):
            p = _dot(_up(WALL[256 + c * 64: 256 + (c + 1) * 64, :]), _up(XN[sl][...]))
            FK[sl][c * 128:c * 128 + 64, :] = _features(p[0:64, :])
            FK[sl][c * 128 + 64:(c + 1) * 128, :] = _features(p[64:128, :])
            yield
        for c in range(4):
            p = _dot(_up(WALL[c * 64:(c + 1) * 64, :]), _up(XN[sl][...]))
            PHQ[i, c * 128:c * 128 + 64, :] = _features(p[0:64, :])
            PHQ[i, c * 128 + 64:(c + 1) * 128, :] = _features(p[64:128, :])
            yield
        for c in range(4):
            p = _dot(_up(WALL[512 + c * 64: 512 + (c + 1) * 64, :]), _up(XN[sl][...]))
            VA[sl][80 * c: 80 * c + 32, :] = _pack2(p[0:32, :], p[32:64, :])
            VA[sl][80 * c + 40: 80 * c + 72, :] = _pack2(p[64:96, :], p[96:128, :])
            yield

    def a1_s3(sl):
        for g in range(8):
            KVA[g] += (_dot_nt(_up(VA[sl][g * 40:(g + 1) * 40, :]),
                               _up(FK[sl][g * 64:(g + 1) * 64, :]))
                       + _dot_nt(_up(VA[sl + 1][g * 40:(g + 1) * 40, :]),
                                 _up(FK[sl + 1][g * 64:(g + 1) * 64, :])))
            yield

    def a_pass1(first, xsrc):
        KVA[...] = jnp.zeros(KVA.shape, F32)
        for sl in (2, 3):
            FK[sl][...] = jnp.zeros(FK[sl].shape, U32)
        if first:
            _interleave((_chain(a1_s0(xsrc, 0, 0), a1_s0(xsrc, 2, 2)), 8))
        _interleave((a1_s1(first, xsrc, 0, 0), 12), (a1_s1(first, xsrc, 1, 1), 12))

        def body(jj, carry):
            def blk(i, sl, nxt):
                p0 = 8 * (2 * jj + sl // 2)
                ex = [(kfft(p0, 2), 2, 0.0, 0.04), (kfft(p0 + 2, 4), 4, 0.42, 0.56),
                      (kfft(p0 + 6, 2), 2, 0.92, 1.0),
                      (a1_s0(xsrc, jnp.minimum(i + 4, NT - 2), sl), 4)] if first else []
                _interleave((a1_s3(2 - sl), 8),
                            (_chain(a1_s2(i, sl), a1_s2(i + 1, sl + 1)), 24),
                            (_chain(a1_s1(first, xsrc, nxt, 2 - sl),
                                    a1_s1(first, xsrc, nxt + 1, 3 - sl)), 24), *ex)

            @pl.when(jj >= 0)
            def _():
                blk(4 * jj, 0, 4 * jj + 2)

            @pl.when(jj >= -1)
            def _():
                blk(4 * jj + 2, 2, jnp.minimum(4 * jj + 4, NT - 2))
            return carry

        lax.fori_loop(0, NT // 4, body, 0)
        _interleave((a1_s3(2), 8))
        r = lax.broadcasted_iota(jnp.int32, (40, 128), 0)
        c = lax.broadcasted_iota(jnp.int32, (40, 128), 1)
        msk = (r % 4) == ((c // 2) % 4)
        for g in range(8):
            KVT[g] = _pack2(jnp.where(msk, KVA[g, pl.ds(0, 40, stride=2), :], 0.0),
                            jnp.where(msk, KVA[g, pl.ds(1, 40, stride=2), :], 0.0))

    def a2_s1(i, sl):
        for g in range(8):
            rr = _dot(_up(KVT[g]), _up(PHQ[i, g * 64:(g + 1) * 64, :]))
            rden = 1.0 / (rr[64:72, :] + 1e-6)
            o = (rr[0:64, :].reshape(8, 8, 128) * rden[None]).reshape(64, 128)
            O[sl][g * 32:(g + 1) * 32, :] = _pack2(o[0:32, :], o[32:64, :])
            yield

    def a2_s2(xsrc, i, sl):
        for c in range(4):
            XT[sl][c * 128:(c + 1) * 128, :] = (
                xsrc[i, c * 128:(c + 1) * 128, :]
                + _dot(_up(WOT[c * 64:(c + 1) * 64, :]), _up(O[sl][...])))
            yield

    def a2_s3(xdst, i, sl):
        def emit(c, w, xe, xo):
            U[i, c * 64:(c + 1) * 64, :] = w
            re = pl.ds(c * 128, 64, stride=2)
            ro = pl.ds(c * 128 + 1, 64, stride=2)
            xdst[i, re, :] = xe + _unpack2(w, 0) * DSK[re, :]
            xdst[i, ro, :] = xo + _unpack2(w, 1) * DSK[ro, :]

        return _ln_gen(lambda c: XT[sl][c * 128:(c + 1) * 128, :],
                       lambda rows: XT[sl][rows, :], emit)

    def a_pass2(xsrc, xdst):
        _interleave((a2_s1(0, 0), 8), (a2_s1(1, 1), 8))

        def body(jj, carry):
            def blk(i, sl, prv0, prv1, nxt):
                _interleave((_chain(a2_s3(xdst, prv0, 2 - sl), a2_s3(xdst, prv1, 3 - sl)), 24),
                            (_chain(a2_s2(xsrc, i, sl), a2_s2(xsrc, i + 1, sl + 1)), 8),
                            (_chain(a2_s1(nxt, 2 - sl), a2_s1(nxt + 1, 3 - sl)), 16))

            @pl.when(jj >= 0)
            def _():
                i = 4 * jj
                blk(i, 0, jnp.where(jj == 0, NT, i - 2), jnp.where(jj == 0, NT, i - 1), i + 2)
                i = 4 * jj + 2
                blk(i, 2, i - 2, i - 1, jnp.minimum(i + 2, NT - 2))
            return carry

        lax.fori_loop(0, NT // 4, body, 0)
        _interleave((a2_s3(xdst, NT - 2, 2), 12), (a2_s3(xdst, NT - 1, 3), 12))

    def b_f(j, par):
        rows = pl.ds(pl.multiple_of(j * (RBK // 2), RBK // 2), RBK // 2)
        pz = ZS[0] + par
        for n in range(8):
            z0 = _dot(_up(U[n, rows, :]), _up(MF[n]))
            z1 = _dot(_up(U[n + 8, rows, :]), _up(MF[n + 8]))
            ZA[pz, n] = z0 + z1
            ZA[pz, n + 8] = z0 - z1
            yield

    def b_m(j, par):
        pz = ZS[1] + par
        for s in range(RBK // 8):
            rr = pl.ds(s * 8, 8)
            kr = pl.ds(pl.multiple_of(j * RBK + s * 8, 8), 8)
            for h in range(2):
                z = [(ZA[pz, 8 * h + n, rr, 0:128], ZA[pz, 8 * h + n, rr, 128:256])
                     for n in range(8)]
                if h:
                    z = [_twiddle(z[n], n, -1) for n in range(8)]
                f = _fft8(z, -1)
                y = [_cmul(f[m], (KF[2 * m + h, kr, 0:128], KF[2 * m + h, kr, 128:256]))
                     for m in range(8)]
                v = _fft8(y, 1)
                if h:
                    v = [_twiddle(v[n], n, 1) for n in range(8)]
                for n in range(8):
                    VB[par][2 * (8 * h + n), rr, :] = v[n][0]
                    VB[par][2 * (8 * h + n) + 1, rr, :] = v[n][1]
                yield

    def b_i(xb, j, vsrc):
        rs = pl.ds(pl.multiple_of(j * RBK, RBK), RBK)
        ev = pl.ds(0, RBK // 2, stride=2)
        od = pl.ds(1, RBK // 2, stride=2)
        pz = ZS[0] + 2
        for n in range(8):
            v0, v1 = [], []
            for c in range(2):
                ee, eo = vsrc[2 * n + c, ev, :], vsrc[2 * n + c, od, :]
                oe, oo = vsrc[2 * n + 16 + c, ev, :], vsrc[2 * n + 16 + c, od, :]
                v0.append(_pack2(ee + oe, eo + oo))
                v1.append(_pack2(ee - oe, eo - oo))
            xb[n, rs, :] += _dot_nt(_up(jnp.concatenate(v0, axis=1)), _up(MF[n]))
            t = xb[n + 8, rs, :] + _dot_nt(_up(jnp.concatenate(v1, axis=1)), _up(MF[n + 8]))
            xb[n + 8, rs, :] = t
            ZA[pz, 0, 0:8, 0:128] = t[RBK - 8:RBK, :]
            yield

    def b_step(gi, gm, gf):
        for k in range(LAG):
            next(gm)
        for k in range(8):
            next(gm, None)
            next(gf)
            next(gm, None)
            next(gi)

    def b_phase(xb, first):
        _interleave((b_f(0, 0), 8))
        VB1[...] = jnp.zeros(VB1.shape, F32)

        def body(jj, carry):
            j = 2 * jj + 1
            b_step(b_i(xb, jnp.maximum(j - 2, 0), VB[1]), b_m(j - 1, 0), b_f(j, 1))

            @pl.when(jj >= 0)
            def _():
                b_step(b_i(xb, j - 1, VB[0]), b_m(j, 1), b_f(jnp.minimum(j + 1, NBK - 1), 0))
            return carry

        lax.fori_loop(0, NBK // 2, body, 0)
        _interleave((b_i(xb, NBK - 1, VB[1]), 8))

    with jax.named_scope("a1"):
        a_pass1(True, XA)
    with jax.named_scope("a2"):
        a_pass2(XA, XB)
    with jax.named_scope("b"):
        b_phase(XB, True)
    with jax.named_scope("a1b"):
        a_pass1(False, XB)
    with jax.named_scope("a2b"):
        a_pass2(XB, XA)
    with jax.named_scope("bb"):
        b_phase(XA, False)
    with jax.named_scope("out"):
        o_cp = [pltpu.make_async_copy(xpb.at[c], out_hbm.at[:, pl.ds(c * 128, 128)], sem.at[c])
                for c in range(4)]
        for c in range(4):
            for m in range(8):
                w = pltpu.pack_elementwise(
                    [XA[2 * m, c * 128:(c + 1) * 128, :], XA[2 * m + 1, c * 128:(c + 1) * 128, :]],
                    packed_dtype=BF16)
                xpu[c, pl.ds(m, 128, stride=8), :] = w.T
            o_cp[c].start()
        for cp in o_cp:
            cp.wait()


@jax.jit
def pallas_interleave_layers__linear_kernel_hedgehog__ssm_conv_s4__prompt_kernel(
    A_x: jax.Array,
    A_wqkv: jax.Array,
    A_w_phi: jax.Array,
    A_wo: jax.Array,
    B_u: jax.Array,
    B_A_re: jax.Array,
    B_A_im: jax.Array,
    B_B_re: jax.Array,
    B_B_im: jax.Array,
    B_C_re: jax.Array,
    B_C_im: jax.Array,
    B_log_dt: jax.Array,
    B_Dskip: jax.Array,
):
    mf = jnp.asarray(_dft_table())
    vm = pl.BlockSpec(memory_space=pltpu.VMEM)
    hb = pl.BlockSpec(memory_space=pl.ANY)
    out = pl.pallas_call(
        _kernel,
        out_shape=jax.ShapeDtypeStruct((S, D), BF16),
        in_specs=[hb, hb, vm, hb, hb, hb, hb, hb, hb, hb, vm, vm, hb],
        out_specs=hb,
        scratch_shapes=[
            pltpu.VMEM((4, S // 2, 128), U32),
            pltpu.VMEM((D // 2, 3 * D), U32),
            pltpu.VMEM((D // 2, D), U32),
            pltpu.VMEM((6, D // 2, NS), U32),
            pltpu.VMEM((NT, 64, 256), U32),
            pltpu.VMEM((NT + 1, D + RBK, 128), F32),
            pltpu.VMEM((NT + 1, D + RBK, 128), F32),
            pltpu.VMEM((NT, D, 256), F32),
            pltpu.VMEM((NT, 512, 128), U32),
            pltpu.VMEM((768, D), U32),
            pltpu.VMEM((256, D), U32),
            pltpu.VMEM((8, 80, 128), F32),
            pltpu.VMEM((8, 40, 128), U32),
            pltpu.VMEM((2, NHI * 2 * EP, 128), U32),
            pltpu.VMEM((2, NHI * 2 * EP, 128), U32),
            pltpu.VMEM((2, NLO * 2 * EP, 128), U32),
            pltpu.VMEM((2, NLO * 2 * EP, 128), U32),
            pltpu.VMEM((4, D, 128), F32),
            pltpu.VMEM((NHI * 4 * PITCH + 136, 128), F32),
            pltpu.VMEM((D, 128), F32),
            pltpu.VMEM((D, 128), F32),
            pltpu.VMEM((NT + 1, 256, 128), U32),
            pltpu.VMEM((3, NT, RBK, 256), F32),
            pltpu.SMEM((2,), jnp.int32),
            pltpu.VMEM((2 * NT, RBK, 128), F32),
            pltpu.VMEM((2 * NT, RBK, 128), F32),
            pltpu.SemaphoreType.DMA((13,)),
        ] + [pltpu.VMEM((256, 128), U32)] * 4
          + [pltpu.VMEM((512, 128), U32)] * 4
          + [pltpu.VMEM((320, 128), U32)] * 4
          + [pltpu.VMEM((256, 128), U32)] * 4
          + [pltpu.VMEM((D, 128), F32)] * 4,
        compiler_params=pltpu.CompilerParams(vmem_limit_bytes=110 * 1024 * 1024),
    )(A_x.reshape(S, D), A_wqkv, A_w_phi, A_wo,
      B_A_re, B_A_im, B_B_re, B_B_im, B_C_re, B_C_im,
      B_log_dt, B_Dskip, mf)
    return out.reshape(1, S, D)
```

```python
import numpy as np
import jax
import jax.numpy as jnp
from jax import lax
import jax.experimental.pallas as pl
import jax.experimental.pallas.tpu as pltpu

F32 = jnp.float32
BF16 = jnp.bfloat16
U32 = jnp.uint32

S = 2048
D = 512
NT = 16
NS = 128
LOG2E = 1.4426950408889634

_R1 = [0, 0, 2, 4, 4, 4, 6, 8, 8, 8, 10, 12, 12, 12, 14, 16]
_R2 = [0, 0, 0, 4, 4, 4, 8, 8, 8, 8, 8, 12, 12, 12, 16, 16]
_R3 = [0, 0, 0, 0, 0, 8, 8, 8, 8, 8, 8, 8, 16, 16, 16, 16]
_HI = ([(0, r) for r in range(17)] + [(1, r) for r in (0, 4, 8, 12, 16)]
       + [(2, r) for r in (0, 8, 16)] + [(3, r) for r in (0, 8, 16)])
_HI_IDX = {qr: i for i, qr in enumerate(_HI)}
NHI = len(_HI)
NLO = 32
GB = 16
EP = 2 * GB + 1
PITCH = 129


def _dft_table():
    n1 = np.arange(16, dtype=np.float64)[:, None, None]
    n2 = np.arange(128, dtype=np.float64)[None, :, None]
    k2 = np.arange(128, dtype=np.float64)[None, None, :]
    th = 2.0 * np.pi * (n1 + 16.0 * n2) * (k2 + 0.5) / 4096.0
    tab = np.concatenate([np.cos(th), -np.sin(th)], axis=2).astype(np.float32)
    bits = tab.astype(BF16).view(np.uint16).astype(np.uint32)
    return bits[:, 0::2, :] | (bits[:, 1::2, :] << 16)


def _cmul(a, b):
    return (a[0] * b[0] - a[1] * b[1], a[0] * b[1] + a[1] * b[0])


def _csq(a):
    return (a[0] * a[0] - a[1] * a[1], (a[0] + a[0]) * a[1])


def _sincos(x):
    big = 12582912.0
    kf = x * 0.6366197723675814 + big
    ki = pltpu.bitcast(kf, jnp.int32)
    k = kf - big
    r = x - k * 1.5703125
    r = r - k * 4.837512969970703125e-4
    r = r - k * 7.54978995489188216e-8
    r = jnp.minimum(jnp.maximum(r, -1.0), 1.0)
    z = r * r
    ps = ((-1.9515295891e-4 * z + 8.3321608736e-3) * z - 1.6666654611e-1) * z * r + r
    pc = (((2.443315711809948e-5 * z - 1.388731625493765e-3) * z + 4.166664568298827e-2) * z
          - 0.5) * z + 1.0
    odd = (ki & 1) == 1
    sn = jnp.where(odd, pc, ps)
    cs = jnp.where(odd, ps, pc)
    sgs = (ki & 2) << 30
    sgc = ((ki + 1) & 2) << 30
    sn = pltpu.bitcast(pltpu.bitcast(sn, jnp.int32) ^ sgs, F32)
    cs = pltpu.bitcast(pltpu.bitcast(cs, jnp.int32) ^ sgc, F32)
    return sn, cs


def _bfly4(x0, x1, x2, x3, sgn):
    a = (x0[0] + x2[0], x0[1] + x2[1])
    b = (x0[0] - x2[0], x0[1] - x2[1])
    c = (x1[0] + x3[0], x1[1] + x3[1])
    d = (x1[0] - x3[0], x1[1] - x3[1])
    y0 = (a[0] + c[0], a[1] + c[1])
    y2 = (a[0] - c[0], a[1] - c[1])
    if sgn < 0:
        y1 = (b[0] + d[1], b[1] - d[0])
        y3 = (b[0] - d[1], b[1] + d[0])
    else:
        y1 = (b[0] - d[1], b[1] + d[0])
        y3 = (b[0] + d[1], b[1] - d[0])
    return y0, y1, y2, y3


def _twiddle(x, m, sgn):
    m = m % 16
    if m == 0:
        return x
    if m == 4:
        return (x[1], -x[0]) if sgn < 0 else (-x[1], x[0])
    c = float(np.cos(2 * np.pi * m / 16))
    s = float(sgn * np.sin(2 * np.pi * m / 16))
    if m in (2, 6):
        h = float(np.sqrt(0.5))
        sc = 1.0 if c > 0 else -1.0
        ss = 1.0 if s > 0 else -1.0
        if sc * ss > 0:
            re = x[0] - x[1]
            im = x[0] + x[1]
            return (re * (h * sc), im * (h * sc))
        re = x[0] + x[1]
        im = x[1] - x[0]
        return (re * (h * sc), im * (h * sc))
    return (x[0] * c - x[1] * s, x[0] * s + x[1] * c)


def _fft16(x, sgn):
    t = [[None] * 4 for _ in range(4)]
    for b in range(4):
        y = _bfly4(x[b], x[4 + b], x[8 + b], x[12 + b], sgn)
        for c in range(4):
            t[b][c] = _twiddle(y[c], b * c, sgn)
    out = [None] * 16
    for c in range(4):
        y = _bfly4(t[0][c], t[1][c], t[2][c], t[3][c], sgn)
        for e in range(4):
            out[c + 4 * e] = y[e]
    return out


def _fft8(x, sgn):
    a = [(x[n][0] + x[n + 4][0], x[n][1] + x[n + 4][1]) for n in range(4)]
    b = [_twiddle((x[n][0] - x[n + 4][0], x[n][1] - x[n + 4][1]), 2 * n, sgn) for n in range(4)]
    ya = _bfly4(a[0], a[1], a[2], a[3], sgn)
    yb = _bfly4(b[0], b[1], b[2], b[3], sgn)
    out = [None] * 8
    for m in range(4):
        out[2 * m] = ya[m]
        out[2 * m + 1] = yb[m]
    return out


def _dot(a, b):
    return jnp.dot(a, b, preferred_element_type=F32)


def _dot_nt(a, b):
    return lax.dot_general(a, b, (((1,), (1,)), ((), ())), preferred_element_type=F32)


def _layernorm_t(xt):
    m = jnp.sum(xt, axis=0, keepdims=True) * (1.0 / D)
    xc = xt - m
    v = jnp.sum(xc * xc, axis=0, keepdims=True) * (1.0 / D)
    return xc * lax.rsqrt(v + 1e-5)


def _pk(x):
    return pltpu.bitcast(x, U32)


def _up(w):
    return pltpu.bitcast(w, BF16)


def _pack2(a, b):
    return pltpu.pack_elementwise([a, b], packed_dtype=BF16)


def _unpack2(w, i):
    return pltpu.unpack_elementwise(w, index=i, packed_dtype=BF16, unpacked_dtype=F32)


def _features(p):
    p3 = p.reshape(8, 8, 128)
    mx = jnp.max(p3, axis=0)
    mx = jnp.maximum(mx, pltpu.roll(mx, 4, 0))
    mn = jnp.min(p3, axis=0)
    mn = jnp.minimum(mn, pltpu.roll(mn, 4, 0))
    ep = jnp.exp2(p3 - mx[None])
    en = jnp.exp2(mn[None] - p3)
    sp = jnp.sum(ep, axis=0)
    sn = jnp.sum(en, axis=0)
    rp = 1.0 / (sp + pltpu.roll(sp, 4, 0))
    rn = 1.0 / (sn + pltpu.roll(sn, 4, 0))
    return _pack2((ep * rp[None]).reshape(64, 128), (en * rn[None]).reshape(64, 128))


def _interleave(*stages):
    order = []
    for i, st in enumerate(stages):
        lo, hi = st[2:] if len(st) > 2 else (0.0, 1.0)
        order += [(lo + (hi - lo) * (k + 0.5) / st[1], i) for k in range(st[1])]
    for _, i in sorted(order):
        next(stages[i][0], None)
    for st in stages:
        for _ in st[0]:
            pass


def _colsum8(x):
    return jnp.sum(x.reshape(x.shape[0] // 8, 8, 128), axis=0)


def _ln_gen(first_pass, load, emit):
    s = None
    for c in range(4):
        t = _colsum8(first_pass(c))
        s = t if s is None else s + t
        yield
    m = jnp.sum(s, axis=0, keepdims=True) * (1.0 / D)
    v = None
    for c in range(4):
        xc = load(pl.ds(c * 128, 128)) - m
        t = _colsum8(xc * xc)
        v = t if v is None else v + t
        yield
    r = lax.rsqrt(jnp.sum(v, axis=0, keepdims=True) * (1.0 / D) + 1e-5)
    for c in range(4):
        xe = load(pl.ds(c * 128, 64, stride=2))
        xo = load(pl.ds(c * 128 + 1, 64, stride=2))
        emit(c, _pack2((xe - m) * r, (xo - m) * r), xe, xo)
        yield


MME = 1.0
ES = 0.0
RBK = 64
NBK = D // RBK


def _kernel(x_hbm, wqkv_hbm, wphi_ref, wo_hbm, are_hbm, aim_hbm, bre_hbm, bim_hbm,
            cre_hbm, cim_hbm, ldt_ref, dsk_ref, mf_hbm, out_hbm,
            XP, WQ, WO, SSM, MF, XA, XB, KF, PHQ, WALL, WOT, KVA, KVT, EH0, EH1, EL0, EL1, EW, KS, DSK, DT,
            U, ZA0, ZA1, VB0, VB1, BD, sem, wsem, *bufs):
    XN, FK, VA, O, XT = [bufs[4 * k:4 * k + 4] for k in range(5)]
    VB = (VB0, VB1)
    ZA = (ZA0, ZA1)
    EHS, ELS = (EH0, EH1), (EL0, EL1)
    lane128 = lax.broadcasted_iota(jnp.int32, (128, 128), 1)
    row128 = lax.broadcasted_iota(jnp.int32, (128, 128), 0)

    ssm_cp = [pltpu.make_async_copy(h, SSM.bitcast(BF16).at[k], sem.at[k])
              for k, h in enumerate((are_hbm, aim_hbm, bre_hbm, bim_hbm, cre_hbm, cim_hbm))]
    mf_cp = pltpu.make_async_copy(mf_hbm, MF, sem.at[6])
    wqb, wob = WQ.bitcast(BF16), WO.bitcast(BF16)

    def w_cp(g):
        off = pl.multiple_of(g * 128, 128)
        return [pltpu.make_async_copy(wqkv_hbm.at[:, pl.ds(p * D + off, 128)], wqb.at[4 * p + g],
                                      wsem.at[g, p]) for p in range(3)]

    wo_cp = [pltpu.make_async_copy(wo_hbm.at[pl.ds(g * 128, 128), :], wob.at[g], wsem.at[g, 3])
             for g in range(4)]
    xpb = XP.bitcast(BF16)
    x_cp = [pltpu.make_async_copy(x_hbm.at[:, pl.ds(c * 128, 128)], xpb.at[c], sem.at[7 + c])
            for c in range(4)]
    for cp in ssm_cp + wo_cp + w_cp(0):
        cp.start()

    with jax.named_scope("kgen_e"):
        dtb = jnp.exp(ldt_ref[...].reshape(1, D).astype(F32)).astype(BF16).astype(F32)
        DT[...] = jnp.broadcast_to(dtb, (128, D)).T
        DSK[...] = jnp.broadcast_to(dsk_ref[...].reshape(1, D).astype(F32), (128, D)).T

        def hd_fe(f):
            return (f // 64) * 4 + f % 4, 2 * ((f % 64) // 8) + (f % 8) // 4

        hd, fe = hd_fe(2 * (row128 % 64) + row128 // 64)
        t = _pk(jnp.where((lane128 // 16 == hd) & (lane128 % 16 == fe), 1.0, 0.0).astype(BF16))
        for k in range(2, 6):
            BD[k, 4] = t
        r256 = lax.broadcasted_iota(jnp.int32, (128, 256), 0)
        c256 = lax.broadcasted_iota(jnp.int32, (128, 256), 1)
        e2t = jnp.where(c256 % 16 == hd_fe(2 * (r256 % 64) + r256 // 64)[1], 1.0, 0.0).astype(BF16)
        hsel = (lax.broadcasted_iota(jnp.int32, (128, 32), 1)
                - lax.broadcasted_iota(jnp.int32, (128, 32), 0) // 16)
        for g in range(4):
            z = _dot_nt(jnp.where(hsel == 8 * g, 1.0, 0.0).astype(BF16), wphi_ref[...])
            z = jnp.where(c256 // 16 == r256 % 16, z, 0.0).astype(BF16)
            t = _pk(jnp.where(lane128 // 16 == hd, _dot_nt(e2t, z), 0.0).astype(BF16))
            for k in range(6):
                BD[k, g] = t
        k6 = lane128 % 64
        r6 = 32 * (k6 % 2) + k6 // 2
        a6 = 32 * (r6 % 2) + r6 // 2
        t = _pk(jnp.where(((row128 // 16) == (lane128 // 64) * 4 + a6 % 4)
                          & (row128 % 16 == 2 * (a6 // 8) + (a6 % 8) // 4), 1.0, 0.0).astype(BF16))
        for k in range(16):
            BD[k // 4, 5 + k % 4] = t
        for b in range(4):
            VA[b][...] = jnp.full(VA[b].shape, 0x3F803F80, U32)
        for cp in ssm_cp:
            cp.wait()
        for cp in w_cp(1) + w_cp(2) + w_cp(3) + x_cp + [mf_cp]:
            cp.start()


    with jax.named_scope("kgen_e1"):
        def e1body(i, carry):
            hr = pl.ds(pl.multiple_of(i * 16, 16), 16)
            raw = [SSM[k, hr, :] for k in range(6)]
            for par in range(2):
                dt = DT[pl.ds(i * 32 + par, 16, stride=2), :]
                prm = [_unpack2(raw[k], par) for k in range(6)]
                dts = dt * (2.0 / 4096.0)
                c0 = _cmul((prm[4], prm[5]), (dts * prm[2], dts * prm[3]))
                mag = jnp.exp(dt * prm[0])
                sn, cs = _sincos(dt * prm[1])
                for k, v in enumerate((mag * cs, mag * sn, c0[0], c0[1])):
                    for h in range(2):
                        EW[k, pl.ds(pl.multiple_of(i * 32 + 16 * h + 8 * par, 8), 8), :] = (
                            v[8 * h:8 * h + 8, :])
            return carry

        lax.fori_loop(0, D // 32, e1body, 0)

    def e_piece(blk, dd, hf, par):
        rows = pl.ds(pl.multiple_of(dd * 128 + blk * GB + 8 * hf, 8), 8)
        EH, EL = EHS[par], ELS[par]
        w = {1: (EW[0, rows, :], EW[1, rows, :])}
        c = {0: (EW[2, rows, :], EW[3, rows, :])}

        def put(ref, n, k, u, v):
            rr = pl.ds((dd * n + k) * EP + 16 * hf, 8, stride=2)
            for cc in range(2):
                ref[cc, rr, :] = _pack2(u[cc], v[cc])

        for b in (1, 2, 4, 8):
            w[2 * b] = _csq(w[b])
            for r in range(b):
                c[r + b] = _cmul(c[r], w[b])
            if b == 1:
                put(EH, NHI // 2, 0, c[0], c[1])
            else:
                for r in range(b, 2 * b, 2):
                    put(EH, NHI // 2, r // 2, c[r], c[r + 1])
            if b >= 4:
                yield
        c[16] = _cmul(c[0], w[16])
        lo = {0: (jnp.ones((8, 128), F32), jnp.zeros((8, 128), F32))}
        for b in (1, 2, 4, 8, 16):
            w[32 * b] = _csq(w[16 * b])
            for j in range(b):
                lo[j + b] = w[16 * b] if j == 0 else _cmul(lo[j], w[16 * b])
                if b == 1:
                    put(EL, NLO // 2, 0, lo[0], lo[1])
                elif j % 2:
                    put(EL, NLO // 2, (j + b) // 2, lo[j + b - 1], lo[j + b])
                if b == 16 and j == 7:
                    yield
            if b >= 4:
                yield
        w[1024] = _csq(w[512])
        w[1536] = _cmul(w[1024], w[512])
        hi = [c[r] if q == 0 else _cmul(c[r], w[512 * q]) for q, r in _HI[16:]]
        for k in range(6):
            put(EH, NHI // 2, 8 + k, hi[2 * k], hi[2 * k + 1])
        yield

    def e_blk(blk, par):
        for hf in range(GB // 8):
            for dd in range(4):
                yield from e_piece(blk, dd, hf, par)

    def mm_blk(blk, par):
        for g in range(GB):
            t = [_dot_nt(_up(EHS[par][c, pl.ds(2 * g, NHI * 2, stride=EP), :]),
                         _up(ELS[par][c, pl.ds(2 * g, NLO * 2, stride=EP), :])) for c in range(2)]
            KS[pl.ds(2 * GB * blk + 2 * g, NHI * 4, stride=PITCH), :] = t[0] - t[1]
            yield

    def wprep(g, parts):
        for q in parts:
            p, c = divmod(q, 4)
            if True:
                if p < 3:
                    t = _dot_nt(_up(BD[q % 6, g] if p < 2 else BD[q % 6, 4]),
                                _up(WQ[4 * p + g, c * 64:(c + 1) * 64, :]))
                    if p < 2:
                        t = t * LOG2E
                    WALL[pl.ds(pl.multiple_of(p * 256 + g * 64, 64), 64),
                         c * 128:(c + 1) * 128] = _pack2(t[0:64, :], t[64:128, :])
                else:
                    wot = _up(WO[g, :, c * 128:(c + 1) * 128]).astype(F32).T.astype(BF16)
                    WOT[g, c * 64:(c + 1) * 64, :] = _pk(_dot(wot, _up(BD[g, 5 + c])).astype(BF16))
                yield

    def _chain(*gens):
        for g in gens:
            yield from g

    with jax.named_scope("kgen_e2"):
        for cp in wo_cp:
            cp.wait()
        _interleave((e_blk(0, 0), 56), (_chain(*[wprep(g, range(12, 16)) for g in range(4)]), 16))

        def ebody(jj, carry):
            for cp in w_cp(jj):
                cp.wait()
            im = [jnp.maximum(2 * jj + k, -1) for k in range(2)]
            ie = [jnp.maximum(2 * jj + 1, -2), jnp.minimum(2 * jj + 2, 128 // GB - 1)]
            iw = jnp.maximum(jj, -3)

            @pl.when(jj >= -1)
            def _():
                _interleave((mm_blk(im[0], 0), GB, 0.0, MME), (e_blk(ie[0], 1), 28 * GB // 8, ES, 1.0),
                            (wprep(iw, range(0, 6)), 6, 0.0, MME))

            @pl.when(jj >= 0)
            def _():
                _interleave((mm_blk(im[1], 1), GB, 0.0, MME), (e_blk(ie[1], 0), 28 * GB // 8, ES, 1.0),
                            (wprep(iw, range(6, 12)), 6, 0.0, MME))
            return carry

        lax.fori_loop(0, 64 // GB, ebody, 0)

    with jax.named_scope("kgen_asm"):
        mf_cp.wait()
        for idx, (q, r) in enumerate(_HI):
            for dd in range(4):
                sh = ((q - dd) * 32) % 128
                if sh:
                    sl = pl.ds((dd * NHI + idx) * PITCH, 128, stride=2)
                    KS[sl, :] = pltpu.roll(KS[sl, :], sh, 1)

        def slab(q, r, dd):
            return KS[pl.ds((dd * NHI + _HI_IDX[(q, r)]) * PITCH, 128, stride=2), :]

        for n1 in range(NT):
            parts = []
            for dd in range(4):
                t = jnp.where(lane128 < 96, slab(2, _R3[n1], dd), slab(3, _R3[n1], dd))
                t = jnp.where(lane128 < 64, slab(1, _R2[n1], dd), t)
                t = jnp.where(lane128 < 32, slab(0, _R1[n1], dd), t)
                t = jnp.where(lane128 < 16, slab(0, n1, dd), t)
                t = t.reshape(8, 16, 128)
                parts.append(_pack2(t[:, 0:8, :], t[:, 8:16, :]).reshape(64, 128))
            kt = jnp.concatenate(parts, axis=0)
            KF[n1] = _dot(_up(kt), _up(MF[n1]))

    def kfft(p0, n):
        for k in range(n):
            rows = pl.ds(pl.multiple_of((p0 + k) * 8, 8), 8)
            z = [(KF[j, rows, 0:128], KF[j, rows, 128:256]) for j in range(NT)]
            f = _fft16(z, -1)
            for j in range(NT):
                KF[j, rows, 0:128] = f[j][0]
                KF[j, rows, 128:256] = f[j][1]
            yield

    for cp in x_cp:
        cp.wait()

    xpu = XP

    def a1_s0(xsrc, i, sl):
        for c in range(4):
            w = xpu[c, pl.ds(i // 2, 128, stride=8), :].T
            for par in range(2):
                XT[sl + par][c * 128:(c + 1) * 128, :] = _unpack2(w, par)
            yield

    def a1_s1(first, xsrc, i, sl):
        def emit(c, w, xe, xo):
            XN[sl][c * 64:(c + 1) * 64, :] = w

        load = (lambda rows: XT[sl][rows, :]) if first else (lambda rows: xsrc[i, rows, :])

        def fp(c):
            xt = load(pl.ds(c * 128, 128))
            if first:
                xsrc[i, c * 128:(c + 1) * 128, :] = xt
            return xt

        return _ln_gen(fp, load, emit)

    def a1_s2(i, sl):
        for c in range(4):
            p = _dot(_up(WALL[256 + c * 64: 256 + (c + 1) * 64, :]), _up(XN[sl][...]))
            FK[sl][c * 128:c * 128 + 64, :] = _features(p[0:64, :])
            FK[sl][c * 128 + 64:(c + 1) * 128, :] = _features(p[64:128, :])
            yield
        for c in range(4):
            p = _dot(_up(WALL[c * 64:(c + 1) * 64, :]), _up(XN[sl][...]))
            PHQ[i, c * 128:c * 128 + 64, :] = _features(p[0:64, :])
            PHQ[i, c * 128 + 64:(c + 1) * 128, :] = _features(p[64:128, :])
            yield
        for c in range(4):
            p = _dot(_up(WALL[512 + c * 64: 512 + (c + 1) * 64, :]), _up(XN[sl][...]))
            VA[sl][80 * c: 80 * c + 32, :] = _pack2(p[0:32, :], p[32:64, :])
            VA[sl][80 * c + 40: 80 * c + 72, :] = _pack2(p[64:96, :], p[96:128, :])
            yield

    def a1_s3(sl):
        for g in range(8):
            KVA[g] += (_dot_nt(_up(VA[sl][g * 40:(g + 1) * 40, :]),
                               _up(FK[sl][g * 64:(g + 1) * 64, :]))
                       + _dot_nt(_up(VA[sl + 1][g * 40:(g + 1) * 40, :]),
                                 _up(FK[sl + 1][g * 64:(g + 1) * 64, :])))
            yield

    def a_pass1(first, xsrc):
        KVA[...] = jnp.zeros(KVA.shape, F32)
        for sl in (2, 3):
            FK[sl][...] = jnp.zeros(FK[sl].shape, U32)
        if first:
            _interleave((_chain(a1_s0(xsrc, 0, 0), a1_s0(xsrc, 2, 2)), 8))
        _interleave((a1_s1(first, xsrc, 0, 0), 12), (a1_s1(first, xsrc, 1, 1), 12))

        def body(jj, carry):
            def blk(sl):
                i = jnp.maximum(4 * jj + sl, 0)
                nxt = jnp.minimum(4 * jj + sl + 2, NT - 2)
                i0 = jnp.minimum(4 * jj + sl + 4, NT - 2)
                p0 = jnp.maximum(16 * jj + 4 * sl, -1)

                @pl.when(jj >= -sl)
                def _():
                    ex = [(kfft(p0, 2), 2, 0.0, 0.04), (kfft(p0 + 2, 4), 4, 0.42, 0.56),
                          (kfft(p0 + 6, 2), 2, 0.92, 1.0),
                          (a1_s0(xsrc, i0, sl), 4)] if first else []
                    _interleave((a1_s3(2 - sl), 8),
                                (_chain(a1_s2(i, sl), a1_s2(i + 1, sl + 1)), 24),
                                (_chain(a1_s1(first, xsrc, nxt, 2 - sl),
                                        a1_s1(first, xsrc, nxt + 1, 3 - sl)), 24), *ex)

            blk(0)
            blk(2)
            return carry

        lax.fori_loop(0, NT // 4, body, 0)
        _interleave((a1_s3(2), 8))
        r = lax.broadcasted_iota(jnp.int32, (40, 128), 0)
        c = lax.broadcasted_iota(jnp.int32, (40, 128), 1)
        msk = (r % 4) == ((c // 2) % 4)
        for g in range(8):
            KVT[g] = _pack2(jnp.where(msk, KVA[g, pl.ds(0, 40, stride=2), :], 0.0),
                            jnp.where(msk, KVA[g, pl.ds(1, 40, stride=2), :], 0.0))

    def a2_s1(i, sl):
        for g in range(8):
            rr = _dot(_up(KVT[g]), _up(PHQ[i, g * 64:(g + 1) * 64, :]))
            rden = 1.0 / (rr[64:72, :] + 1e-6)
            o = (rr[0:64, :].reshape(8, 8, 128) * rden[None]).reshape(64, 128)
            O[sl][g * 32:(g + 1) * 32, :] = _pack2(o[0:32, :], o[32:64, :])
            yield

    def a2_s2(xsrc, i, sl):
        for c in range(4):
            XT[sl][c * 128:(c + 1) * 128, :] = (
                xsrc[i, c * 128:(c + 1) * 128, :]
                + _dot(_up(jnp.concatenate([WOT[g, c * 64:(c + 1) * 64, :] for g in range(4)],
                                           axis=1)), _up(O[sl][...])))
            yield

    def a2_s3(xdst, i, sl):
        def emit(c, w, xe, xo):
            U[i, c * 64:(c + 1) * 64, :] = w
            re = pl.ds(c * 128, 64, stride=2)
            ro = pl.ds(c * 128 + 1, 64, stride=2)
            xdst[i, re, :] = xe + _unpack2(w, 0) * DSK[re, :]
            xdst[i, ro, :] = xo + _unpack2(w, 1) * DSK[ro, :]

        return _ln_gen(lambda c: XT[sl][c * 128:(c + 1) * 128, :],
                       lambda rows: XT[sl][rows, :], emit)

    def a_pass2(xsrc, xdst):
        _interleave((a2_s1(0, 0), 8), (a2_s1(1, 1), 8))

        def body(jj, carry):
            def blk(i, sl, prv0, prv1, nxt):
                _interleave((_chain(a2_s3(xdst, prv0, 2 - sl), a2_s3(xdst, prv1, 3 - sl)), 24),
                            (_chain(a2_s2(xsrc, i, sl), a2_s2(xsrc, i + 1, sl + 1)), 8),
                            (_chain(a2_s1(nxt, 2 - sl), a2_s1(nxt + 1, 3 - sl)), 16))

            i = 4 * jj
            ia = [jnp.maximum(i, -1), jnp.where(jj == 0, NT, i - 2), jnp.where(jj == 0, NT, i - 1),
                  jnp.maximum(i + 2, -2)]
            ib = [jnp.maximum(i + 2, -3), jnp.maximum(i, -4), jnp.maximum(i + 1, -5),
                  jnp.minimum(i + 4, NT - 2)]

            @pl.when(jj >= 0)
            def _():
                blk(ia[0], 0, *ia[1:])
                blk(ib[0], 2, *ib[1:])
            return carry

        lax.fori_loop(0, NT // 4, body, 0)
        _interleave((a2_s3(xdst, NT - 2, 2), 12), (a2_s3(xdst, NT - 1, 3), 12))

    def b_f(j, par):
        rows = pl.ds(pl.multiple_of(j * (RBK // 2), RBK // 2), RBK // 2)
        for n in range(8):
            z0 = _dot(_up(U[n, rows, :]), _up(MF[n]))
            z1 = _dot(_up(U[n + 8, rows, :]), _up(MF[n + 8]))
            ZA[par][n] = z0 + z1
            ZA[par][n + 8] = z0 - z1
            yield

    def b_m(j, par):
        for s in range(RBK // 8):
            rr = pl.ds(s * 8, 8)
            kr = pl.ds(pl.multiple_of(j * RBK + s * 8, 8), 8)
            for h in range(2):
                z = [(ZA[par][8 * h + n, rr, 0:128], ZA[par][8 * h + n, rr, 128:256])
                     for n in range(8)]
                if h:
                    z = [_twiddle(z[n], n, -1) for n in range(8)]
                f = _fft8(z, -1)
                y = [_cmul(f[m], (KF[2 * m + h, kr, 0:128], KF[2 * m + h, kr, 128:256]))
                     for m in range(8)]
                v = _fft8(y, 1)
                if h:
                    v = [_twiddle(v[n], n, 1) for n in range(8)]
                for n in range(8):
                    VB[par][2 * (8 * h + n), rr, :] = v[n][0]
                    VB[par][2 * (8 * h + n) + 1, rr, :] = v[n][1]
                yield

    def b_i(xb, j, vsrc, half=None):
        rs = pl.ds(pl.multiple_of(j * RBK, RBK), RBK)
        ev = pl.ds(0, RBK // 2, stride=2)
        od = pl.ds(1, RBK // 2, stride=2)
        prev = None
        for n in range(8):
            v0, v1 = [], []
            for c in range(2):
                ee, eo = vsrc[2 * n + c, ev, :], vsrc[2 * n + c, od, :]
                oe, oo = vsrc[2 * n + 16 + c, ev, :], vsrc[2 * n + 16 + c, od, :]
                v0.append(_pack2(ee + oe, eo + oo))
                v1.append(_pack2(ee - oe, eo - oo))
            r = [xb[n, rs, :] + _dot_nt(_up(jnp.concatenate(v0, axis=1)), _up(MF[n])),
                 xb[n + 8, rs, :] + _dot_nt(_up(jnp.concatenate(v1, axis=1)), _up(MF[n + 8]))]
            if half is None:
                xb[n, rs, :] = r[0]
                xb[n + 8, rs, :] = r[1]
            elif n % 2:
                for h in range(2):
                    m = n // 2 + 4 * h
                    w = _pack2(prev[h], r[h])
                    if half:
                        w = jnp.concatenate([FK[0][m * RBK:(m + 1) * RBK, :], w], axis=0)
                        xpu[j // 2, pl.ds(m, 128, stride=8), :] = w.T
                    else:
                        FK[0][m * RBK:(m + 1) * RBK, :] = w
            prev = r
            yield

    def b_step(gi, gm, gf):
        for k in range(8):
            next(gf)
            next(gm)
            next(gi)
            next(gm)

    def o_cp(c):
        return pltpu.make_async_copy(
            xpb.at[c], out_hbm.at[:, pl.ds(pl.multiple_of(c * 128, 128), 128)], sem.at[c])

    def b_phase(xb, first):
        _interleave((b_f(0, 0), 8))
        VB1[...] = jnp.zeros(VB1.shape, F32)
        h0, h1 = (None, None) if first else (0, 1)

        def body(jj, carry):
            j = 2 * jj + 1

            @pl.when(jj >= -1)
            def _():
                b_step(b_i(xb, jnp.maximum(j - 2, 0), VB[1], h1), b_m(j - 1, 0), b_f(j, 1))

            if not first:
                @pl.when(jj >= 1)
                def _():
                    o_cp(jj - 1).start()

            @pl.when(jj >= 0)
            def _():
                b_step(b_i(xb, jnp.maximum(j - 1, 0), VB[0], h0), b_m(j, 1),
                       b_f(jnp.minimum(j + 1, NBK - 1), 0))
            return carry

        lax.fori_loop(0, NBK // 2, body, 0)
        _interleave((b_i(xb, NBK - 1, VB[1], h1), 8))

    with jax.named_scope("a1"):
        a_pass1(True, XA)
    with jax.named_scope("a2"):
        a_pass2(XA, XB)
    with jax.named_scope("b"):
        b_phase(XB, True)
    with jax.named_scope("a1b"):
        a_pass1(False, XB)
    with jax.named_scope("a2b"):
        a_pass2(XB, XA)
    with jax.named_scope("bb"):
        b_phase(XA, False)
    with jax.named_scope("out"):
        o_cp(3).start()
        for c in range(4):
            o_cp(c).wait()


@jax.jit
def pallas_interleave_layers__linear_kernel_hedgehog__ssm_conv_s4__prompt_kernel(
    A_x: jax.Array,
    A_wqkv: jax.Array,
    A_w_phi: jax.Array,
    A_wo: jax.Array,
    B_u: jax.Array,
    B_A_re: jax.Array,
    B_A_im: jax.Array,
    B_B_re: jax.Array,
    B_B_im: jax.Array,
    B_C_re: jax.Array,
    B_C_im: jax.Array,
    B_log_dt: jax.Array,
    B_Dskip: jax.Array,
):
    mf = jnp.asarray(_dft_table())
    vm = pl.BlockSpec(memory_space=pltpu.VMEM)
    hb = pl.BlockSpec(memory_space=pl.ANY)
    out = pl.pallas_call(
        _kernel,
        out_shape=jax.ShapeDtypeStruct((S, D), BF16),
        in_specs=[hb, hb, vm, hb, hb, hb, hb, hb, hb, hb, vm, vm, hb],
        out_specs=hb,
        scratch_shapes=[
            pltpu.VMEM((4, S // 2, 128), U32),
            pltpu.VMEM((12, D // 2, 128), U32),
            pltpu.VMEM((4, 64, D), U32),
            pltpu.VMEM((6, D // 2, NS), U32),
            pltpu.VMEM((NT, 64, 256), U32),
            pltpu.VMEM((NT + 1, D + RBK, 128), F32),
            pltpu.VMEM((NT + 1, D + RBK, 128), F32),
            pltpu.VMEM((NT, D, 256), F32),
            pltpu.VMEM((NT, 512, 128), U32),
            pltpu.VMEM((768, D), U32),
            pltpu.VMEM((4, 256, 128), U32),
            pltpu.VMEM((8, 80, 128), F32),
            pltpu.VMEM((8, 40, 128), U32),
            pltpu.VMEM((2, NHI * 2 * EP, 128), U32),
            pltpu.VMEM((2, NHI * 2 * EP, 128), U32),
            pltpu.VMEM((2, NLO * 2 * EP, 128), U32),
            pltpu.VMEM((2, NLO * 2 * EP, 128), U32),
            pltpu.VMEM((4, D, 128), F32),
            pltpu.VMEM((NHI * 4 * PITCH + 136, 128), F32),
            pltpu.VMEM((D, 128), F32),
            pltpu.VMEM((D, 128), F32),
            pltpu.VMEM((NT + 1, 256, 128), U32),
            pltpu.VMEM((NT, RBK, 256), F32),
            pltpu.VMEM((NT, RBK, 256), F32),
            pltpu.VMEM((2 * NT, RBK, 128), F32),
            pltpu.VMEM((2 * NT, RBK, 128), F32),
            pltpu.VMEM((6, 9, 64, 128), U32),
            pltpu.SemaphoreType.DMA((11,)),
            pltpu.SemaphoreType.DMA((4, 4)),
        ] + [pltpu.VMEM((256, 128), U32)] * 4
          + [pltpu.VMEM((512, 128), U32)] * 4
          + [pltpu.VMEM((320, 128), U32)] * 4
          + [pltpu.VMEM((256, 128), U32)] * 4
          + [pltpu.VMEM((D, 128), F32)] * 4,
        compiler_params=pltpu.CompilerParams(vmem_limit_bytes=110 * 1024 * 1024),
    )(A_x.reshape(S, D), A_wqkv, jnp.transpose(A_w_phi, (1, 2, 0)).reshape(256, 32), A_wo,
      B_A_re, B_A_im, B_B_re, B_B_im, B_C_re, B_C_im,
      B_log_dt, B_Dskip, mf)
    return out.reshape(1, S, D)
```

```python
import numpy as np
import jax
import jax.numpy as jnp
from jax import lax
import jax.experimental.pallas as pl
import jax.experimental.pallas.tpu as pltpu

F32 = jnp.float32
BF16 = jnp.bfloat16
U32 = jnp.uint32

S = 2048
D = 512
NT = 16
NS = 128
LOG2E = 1.4426950408889634

_R1 = [0, 0, 2, 4, 4, 4, 6, 8, 8, 8, 10, 12, 12, 12, 14, 16]
_R2 = [0, 0, 0, 4, 4, 4, 8, 8, 8, 8, 8, 12, 12, 12, 16, 16]
_R3 = [0, 0, 0, 0, 0, 8, 8, 8, 8, 8, 8, 8, 16, 16, 16, 16]
_HI = ([(0, r) for r in range(17)] + [(1, r) for r in (0, 4, 8, 12, 16)]
       + [(2, r) for r in (0, 8, 16)] + [(3, r) for r in (0, 8, 16)])
_HI_IDX = {qr: i for i, qr in enumerate(_HI)}
NHI = len(_HI)
NLO = 32
GB = 16
EP = 2 * GB + 1
PITCH = 129


def _dft_table():
    n1 = np.arange(16, dtype=np.float64)[:, None, None]
    n2 = np.arange(128, dtype=np.float64)[None, :, None]
    k2 = np.arange(128, dtype=np.float64)[None, None, :]
    th = 2.0 * np.pi * (n1 + 16.0 * n2) * (k2 + 0.5) / 4096.0
    tab = np.concatenate([np.cos(th), -np.sin(th)], axis=2).astype(np.float32)
    bits = tab.astype(BF16).view(np.uint16).astype(np.uint32)
    return bits[:, 0::2, :] | (bits[:, 1::2, :] << 16)


def _cmul(a, b):
    return (a[0] * b[0] - a[1] * b[1], a[0] * b[1] + a[1] * b[0])


def _csq(a):
    return (a[0] * a[0] - a[1] * a[1], (a[0] + a[0]) * a[1])


def _sincos(x):
    big = 12582912.0
    kf = x * 0.6366197723675814 + big
    ki = pltpu.bitcast(kf, jnp.int32)
    k = kf - big
    r = x - k * 1.5703125
    r = r - k * 4.837512969970703125e-4
    r = r - k * 7.54978995489188216e-8
    r = jnp.minimum(jnp.maximum(r, -1.0), 1.0)
    z = r * r
    ps = ((-1.9515295891e-4 * z + 8.3321608736e-3) * z - 1.6666654611e-1) * z * r + r
    pc = (((2.443315711809948e-5 * z - 1.388731625493765e-3) * z + 4.166664568298827e-2) * z
          - 0.5) * z + 1.0
    odd = (ki & 1) == 1
    sn = jnp.where(odd, pc, ps)
    cs = jnp.where(odd, ps, pc)
    sgs = (ki & 2) << 30
    sgc = ((ki + 1) & 2) << 30
    sn = pltpu.bitcast(pltpu.bitcast(sn, jnp.int32) ^ sgs, F32)
    cs = pltpu.bitcast(pltpu.bitcast(cs, jnp.int32) ^ sgc, F32)
    return sn, cs


def _bfly4(x0, x1, x2, x3, sgn):
    a = (x0[0] + x2[0], x0[1] + x2[1])
    b = (x0[0] - x2[0], x0[1] - x2[1])
    c = (x1[0] + x3[0], x1[1] + x3[1])
    d = (x1[0] - x3[0], x1[1] - x3[1])
    y0 = (a[0] + c[0], a[1] + c[1])
    y2 = (a[0] - c[0], a[1] - c[1])
    if sgn < 0:
        y1 = (b[0] + d[1], b[1] - d[0])
        y3 = (b[0] - d[1], b[1] + d[0])
    else:
        y1 = (b[0] - d[1], b[1] + d[0])
        y3 = (b[0] + d[1], b[1] - d[0])
    return y0, y1, y2, y3


def _twiddle(x, m, sgn):
    m = m % 16
    if m == 0:
        return x
    if m == 4:
        return (x[1], -x[0]) if sgn < 0 else (-x[1], x[0])
    c = float(np.cos(2 * np.pi * m / 16))
    s = float(sgn * np.sin(2 * np.pi * m / 16))
    if m in (2, 6):
        h = float(np.sqrt(0.5))
        sc = 1.0 if c > 0 else -1.0
        ss = 1.0 if s > 0 else -1.0
        if sc * ss > 0:
            re = x[0] - x[1]
            im = x[0] + x[1]
            return (re * (h * sc), im * (h * sc))
        re = x[0] + x[1]
        im = x[1] - x[0]
        return (re * (h * sc), im * (h * sc))
    return (x[0] * c - x[1] * s, x[0] * s + x[1] * c)


def _fft16(x, sgn):
    t = [[None] * 4 for _ in range(4)]
    for b in range(4):
        y = _bfly4(x[b], x[4 + b], x[8 + b], x[12 + b], sgn)
        for c in range(4):
            t[b][c] = _twiddle(y[c], b * c, sgn)
    out = [None] * 16
    for c in range(4):
        y = _bfly4(t[0][c], t[1][c], t[2][c], t[3][c], sgn)
        for e in range(4):
            out[c + 4 * e] = y[e]
    return out


def _fft8(x, sgn):
    a = [(x[n][0] + x[n + 4][0], x[n][1] + x[n + 4][1]) for n in range(4)]
    b = [_twiddle((x[n][0] - x[n + 4][0], x[n][1] - x[n + 4][1]), 2 * n, sgn) for n in range(4)]
    ya = _bfly4(a[0], a[1], a[2], a[3], sgn)
    yb = _bfly4(b[0], b[1], b[2], b[3], sgn)
    out = [None] * 8
    for m in range(4):
        out[2 * m] = ya[m]
        out[2 * m + 1] = yb[m]
    return out


def _dot(a, b):
    return jnp.dot(a, b, preferred_element_type=F32)


def _dot_nt(a, b):
    return lax.dot_general(a, b, (((1,), (1,)), ((), ())), preferred_element_type=F32)


def _layernorm_t(xt):
    m = jnp.sum(xt, axis=0, keepdims=True) * (1.0 / D)
    xc = xt - m
    v = jnp.sum(xc * xc, axis=0, keepdims=True) * (1.0 / D)
    return xc * lax.rsqrt(v + 1e-5)


def _pk(x):
    return pltpu.bitcast(x, U32)


def _up(w):
    return pltpu.bitcast(w, BF16)


def _pack2(a, b):
    return pltpu.pack_elementwise([a, b], packed_dtype=BF16)


def _unpack2(w, i):
    return pltpu.unpack_elementwise(w, index=i, packed_dtype=BF16, unpacked_dtype=F32)


def _features(p):
    p3 = p.reshape(8, 8, 128)
    mx = jnp.max(p3, axis=0)
    mx = jnp.maximum(mx, pltpu.roll(mx, 4, 0))
    mn = jnp.min(p3, axis=0)
    mn = jnp.minimum(mn, pltpu.roll(mn, 4, 0))
    ep = jnp.exp2(p3 - mx[None])
    en = jnp.exp2(mn[None] - p3)
    sp = jnp.sum(ep, axis=0)
    sn = jnp.sum(en, axis=0)
    rp = 1.0 / (sp + pltpu.roll(sp, 4, 0))
    rn = 1.0 / (sn + pltpu.roll(sn, 4, 0))
    return _pack2((ep * rp[None]).reshape(64, 128), (en * rn[None]).reshape(64, 128))


def _interleave(*stages):
    order = []
    for i, st in enumerate(stages):
        lo, hi = st[2:] if len(st) > 2 else (0.0, 1.0)
        order += [(lo + (hi - lo) * (k + 0.5) / st[1], i) for k in range(st[1])]
    for _, i in sorted(order):
        next(stages[i][0], None)
    for st in stages:
        for _ in st[0]:
            pass


def _colsum8(x):
    return jnp.sum(x.reshape(x.shape[0] // 8, 8, 128), axis=0)


def _ln_gen(first_pass, load, emit):
    s = None
    for c in range(4):
        t = _colsum8(first_pass(c))
        s = t if s is None else s + t
        yield
    m = jnp.sum(s, axis=0, keepdims=True) * (1.0 / D)
    v = None
    for c in range(4):
        xc = load(pl.ds(c * 128, 128)) - m
        t = _colsum8(xc * xc)
        v = t if v is None else v + t
        yield
    r = lax.rsqrt(jnp.sum(v, axis=0, keepdims=True) * (1.0 / D) + 1e-5)
    for c in range(4):
        xe = load(pl.ds(c * 128, 64, stride=2))
        xo = load(pl.ds(c * 128 + 1, 64, stride=2))
        emit(c, _pack2((xe - m) * r, (xo - m) * r), xe, xo)
        yield


MME = 1.0
KB = (0.0, 1.0)
KA = (0.0, 1.0)
ES = 0.0
RBK = 64
NBK = D // RBK


def _kernel(x_hbm, wqkv_hbm, wphi_ref, wo_hbm, are_hbm, aim_hbm, bre_hbm, bim_hbm,
            cre_hbm, cim_hbm, ldt_ref, dsk_ref, mf_hbm, out_hbm,
            XP, WQ, WO, SSM, MF, XA, XB, KF, PHQ, WALL, WOT, KVA, KVT, EH0, EH1, EL0, EL1, EW, KS, DSK, DT,
            U, ZA0, ZA1, VB0, VB1, BD, sem, wsem, *bufs):
    XN, FK, VA, O, XT = [bufs[4 * k:4 * k + 4] for k in range(5)]
    VB = (VB0, VB1)
    ZA = (ZA0, ZA1)
    EHS, ELS = (EH0, EH1), (EL0, EL1)
    lane128 = lax.broadcasted_iota(jnp.int32, (128, 128), 1)
    row128 = lax.broadcasted_iota(jnp.int32, (128, 128), 0)

    ssm_cp = [pltpu.make_async_copy(h, SSM.bitcast(BF16).at[k], sem.at[k])
              for k, h in enumerate((are_hbm, aim_hbm, bre_hbm, bim_hbm, cre_hbm, cim_hbm))]
    mf_cp = pltpu.make_async_copy(mf_hbm, MF, sem.at[6])
    wqb, wob = WQ.bitcast(BF16), WO.bitcast(BF16)

    def w_cp(g):
        off = pl.multiple_of(g * 128, 128)
        return [pltpu.make_async_copy(wqkv_hbm.at[:, pl.ds(p * D + off, 128)], wqb.at[4 * p + g],
                                      wsem.at[g, p]) for p in range(3)]

    wo_cp = [pltpu.make_async_copy(wo_hbm.at[pl.ds(g * 128, 128), :], wob.at[g], wsem.at[g, 3])
             for g in range(4)]
    xpb = XP.bitcast(BF16)
    x_cp = [pltpu.make_async_copy(x_hbm.at[:, pl.ds(c * 128, 128)], xpb.at[c], sem.at[7 + c])
            for c in range(4)]
    for cp in ssm_cp + wo_cp + w_cp(0):
        cp.start()

    with jax.named_scope("kgen_e"):
        dtb = jnp.exp(ldt_ref[...].reshape(1, D).astype(F32)).astype(BF16).astype(F32)
        DT[...] = jnp.broadcast_to(dtb, (128, D)).T
        DSK[...] = jnp.broadcast_to(dsk_ref[...].reshape(1, D).astype(F32), (128, D)).T

        def hd_fe(f):
            return (f // 64) * 4 + f % 4, 2 * ((f % 64) // 8) + (f % 8) // 4

        hd, fe = hd_fe(2 * (row128 % 64) + row128 // 64)
        t = _pk(jnp.where((lane128 // 16 == hd) & (lane128 % 16 == fe), 1.0, 0.0).astype(BF16))
        for k in range(2, 6):
            BD[k, 4] = t
        r256 = lax.broadcasted_iota(jnp.int32, (128, 256), 0)
        c256 = lax.broadcasted_iota(jnp.int32, (128, 256), 1)
        e2t = jnp.where(c256 % 16 == hd_fe(2 * (r256 % 64) + r256 // 64)[1], 1.0, 0.0).astype(BF16)
        hsel = (lax.broadcasted_iota(jnp.int32, (128, 32), 1)
                - lax.broadcasted_iota(jnp.int32, (128, 32), 0) // 16)
        for g in range(4):
            z = _dot_nt(jnp.where(hsel == 8 * g, 1.0, 0.0).astype(BF16), wphi_ref[...])
            z = jnp.where(c256 // 16 == r256 % 16, z, 0.0).astype(BF16)
            t = _pk(jnp.where(lane128 // 16 == hd, _dot_nt(e2t, z), 0.0).astype(BF16))
            for k in range(6):
                BD[k, g] = t
        k6 = lane128 % 64
        r6 = 32 * (k6 % 2) + k6 // 2
        a6 = 32 * (r6 % 2) + r6 // 2
        t = _pk(jnp.where(((row128 // 16) == (lane128 // 64) * 4 + a6 % 4)
                          & (row128 % 16 == 2 * (a6 // 8) + (a6 % 8) // 4), 1.0, 0.0).astype(BF16))
        for k in range(16):
            BD[k // 4, 5 + k % 4] = t
        for b in range(4):
            VA[b][...] = jnp.full(VA[b].shape, 0x3F803F80, U32)
        for cp in ssm_cp:
            cp.wait()
        for cp in w_cp(1) + w_cp(2) + w_cp(3) + x_cp + [mf_cp]:
            cp.start()


    with jax.named_scope("kgen_e1"):
        def e1body(i, carry):
            hr = pl.ds(pl.multiple_of(i * 16, 16), 16)
            raw = [SSM[k, hr, :] for k in range(6)]
            for par in range(2):
                dt = DT[pl.ds(i * 32 + par, 16, stride=2), :]
                prm = [_unpack2(raw[k], par) for k in range(6)]
                dts = dt * (2.0 / 4096.0)
                c0 = _cmul((prm[4], prm[5]), (dts * prm[2], dts * prm[3]))
                mag = jnp.exp(dt * prm[0])
                sn, cs = _sincos(dt * prm[1])
                for k, v in enumerate((mag * cs, mag * sn, c0[0], c0[1])):
                    for h in range(2):
                        EW[k, pl.ds(pl.multiple_of(i * 32 + 16 * h + 8 * par, 8), 8), :] = (
                            v[8 * h:8 * h + 8, :])
            return carry

        lax.fori_loop(0, D // 32, e1body, 0)

    def e_piece(blk, dd, hf, par):
        rows = pl.ds(pl.multiple_of(dd * 128 + blk * GB + 8 * hf, 8), 8)
        EH, EL = EHS[par], ELS[par]
        w = {1: (EW[0, rows, :], EW[1, rows, :])}
        c = {}

        def put(ref, n, k, u, v):
            rr = pl.ds((dd * n + k) * EP + 16 * hf, 8, stride=2)
            for cc in range(2):
                ref[cc, rr, :] = _pack2(u[cc], v[cc])

        for b in (1, 2, 4, 8, 16, 32):
            w[2 * b] = _csq(w[b])
        lo = {0: (jnp.ones((8, 128), F32), jnp.zeros((8, 128), F32)), 1: w[16], 2: w[32],
              3: _cmul(w[16], w[32]), 4: w[64]}
        for j in range(NLO):
            if j > 4:
                lo[j] = _cmul(lo[j - 4], w[64])
            if j % 2:
                put(EL, NLO // 2, j // 2, lo[j - 1], lo[j])
            if j % 8 == 7:
                yield
        w[512] = _cmul(lo[28], w[64])
        w[1024] = _csq(w[512])
        w[1536] = _cmul(w[1024], w[512])
        c[0] = (EW[2, rows, :], EW[3, rows, :])
        for r in range(1, 17):
            c[r] = (_cmul(c[r - 4], w[4]) if r >= 4 else
                    _cmul(c[1], w[2]) if r == 3 else _cmul(c[0], w[r]))
            if r % 2:
                put(EH, NHI // 2, r // 2, c[r - 1], c[r])
            if r % 8 == 7:
                yield
        hi = [c[r] if q == 0 else _cmul(c[r], w[512 * q]) for q, r in _HI[16:]]
        for k in range(6):
            put(EH, NHI // 2, 8 + k, hi[2 * k], hi[2 * k + 1])
        yield

    def e_blk(blk, par):
        for hf in range(GB // 8):
            for dd in range(4):
                yield from e_piece(blk, dd, hf, par)

    def mm_blk(blk, par):
        for g in range(GB):
            t = [_dot_nt(_up(EHS[par][c, pl.ds(2 * g, NHI * 2, stride=EP), :]),
                         _up(ELS[par][c, pl.ds(2 * g, NLO * 2, stride=EP), :])) for c in range(2)]
            KS[pl.ds(2 * GB * blk + 2 * g, NHI * 4, stride=PITCH), :] = t[0] - t[1]
            yield

    def wprep(g, parts):
        for q in parts:
            p, c = divmod(q, 4)
            if True:
                if p < 3:
                    t = _dot_nt(_up(BD[q % 6, g] if p < 2 else BD[q % 6, 4]),
                                _up(WQ[4 * p + g, c * 64:(c + 1) * 64, :]))
                    if p < 2:
                        t = t * LOG2E
                    WALL[pl.ds(pl.multiple_of(p * 256 + g * 64, 64), 64),
                         c * 128:(c + 1) * 128] = _pack2(t[0:64, :], t[64:128, :])
                else:
                    wot = _up(WO[g, :, c * 128:(c + 1) * 128]).astype(F32).T.astype(BF16)
                    WOT[g, c * 64:(c + 1) * 64, :] = _pk(_dot(wot, _up(BD[g, 5 + c])).astype(BF16))
                yield

    def _chain(*gens):
        for g in gens:
            yield from g

    with jax.named_scope("kgen_e2"):
        for cp in wo_cp:
            cp.wait()
        _interleave((e_blk(0, 0), 56), (_chain(*[wprep(g, range(12, 16)) for g in range(4)]), 16))

        def ebody(jj, carry):
            for cp in w_cp(jj):
                cp.wait()
            im = [jnp.maximum(2 * jj + k, -1) for k in range(2)]
            ie = [jnp.maximum(2 * jj + 1, -2), jnp.minimum(2 * jj + 2, 128 // GB - 1)]
            iw = jnp.maximum(jj, -3)

            @pl.when(jj >= -1)
            def _():
                _interleave((mm_blk(im[0], 0), GB, 0.0, MME), (e_blk(ie[0], 1), 28 * GB // 8, ES, 1.0),
                            (wprep(iw, range(0, 6)), 6, 0.0, MME))

            @pl.when(jj < 64 // GB - 1)
            def _():
                _interleave((mm_blk(im[1], 1), GB, 0.0, MME), (e_blk(ie[1], 0), 28 * GB // 8, ES, 1.0),
                            (wprep(iw, range(6, 12)), 6, 0.0, MME))

            @pl.when(jj == 64 // GB - 1)
            def _():
                _interleave((mm_blk(im[1], 1), GB), (wprep(iw, range(6, 12)), 6))
            return carry

        lax.fori_loop(0, 64 // GB, ebody, 0)

    with jax.named_scope("kgen_asm"):
        mf_cp.wait()
        def rolls(dd):
            for idx, (q, r) in enumerate(_HI):
                sh = ((q - dd) * 32) % 128
                if sh:
                    sl = pl.ds((dd * NHI + idx) * PITCH, 128, stride=2)
                    KS[sl, :] = pltpu.roll(KS[sl, :], sh, 1)
                    yield

        def slab(q, r, dd):
            return KS[pl.ds((dd * NHI + _HI_IDX[(q, r)]) * PITCH, 128, stride=2), :]

        def kpart(n1, dd):
            t = jnp.where(lane128 < 96, slab(2, _R3[n1], dd), slab(3, _R3[n1], dd))
            t = jnp.where(lane128 < 64, slab(1, _R2[n1], dd), t)
            t = jnp.where(lane128 < 32, slab(0, _R1[n1], dd), t)
            t = jnp.where(lane128 < 16, slab(0, n1, dd), t)
            t = t.reshape(8, 16, 128)
            return _dot(_up(_pack2(t[:, 0:8, :], t[:, 8:16, :]).reshape(64, 128)), _up(MF[n1]))

        def asm(dd):
            for n1 in range(8):
                z0, z1 = kpart(n1, dd), kpart(n1 + 8, dd)
                KF[n1, dd * 128:(dd + 1) * 128, :] = z0 + z1
                KF[n1 + 8, dd * 128:(dd + 1) * 128, :] = z0 - z1
                yield

        _interleave((rolls(0), 11))
        for dd in range(4):
            _interleave((asm(dd), 8), *([(rolls(dd + 1), 25)] if dd < 3 else []))

    def kfft(p0, n):
        for k in range(n):
            rows = pl.ds(pl.multiple_of((p0 + k) * 8, 8), 8)
            for h in range(2):
                z = [(KF[8 * h + j, rows, 0:128], KF[8 * h + j, rows, 128:256]) for j in range(8)]
                if h:
                    z = [_twiddle(z[j], j, -1) for j in range(8)]
                f = _fft8(z, -1)
                for j in range(8):
                    KF[8 * h + j, rows, 0:128] = f[j][0]
                    KF[8 * h + j, rows, 128:256] = f[j][1]
                yield

    for cp in x_cp:
        cp.wait()

    xpu = XP

    def a1_s0(xsrc, i, sl):
        for c in range(4):
            w = xpu[c, pl.ds(i // 2, 128, stride=8), :].T
            for par in range(2):
                XT[sl + par][c * 128:(c + 1) * 128, :] = _unpack2(w, par)
            yield

    def a1_s1(first, xsrc, i, sl):
        def emit(c, w, xe, xo):
            XN[sl][c * 64:(c + 1) * 64, :] = w

        load = (lambda rows: XT[sl][rows, :]) if first else (lambda rows: xsrc[i, rows, :])

        def fp(c):
            xt = load(pl.ds(c * 128, 128))
            if first:
                xsrc[i, c * 128:(c + 1) * 128, :] = xt
            return xt

        return _ln_gen(fp, load, emit)

    def a1_s2(i, sl):
        for c in range(4):
            p = _dot(_up(WALL[256 + c * 64: 256 + (c + 1) * 64, :]), _up(XN[sl][...]))
            FK[sl][c * 128:c * 128 + 64, :] = _features(p[0:64, :])
            FK[sl][c * 128 + 64:(c + 1) * 128, :] = _features(p[64:128, :])
            yield
        for c in range(4):
            p = _dot(_up(WALL[c * 64:(c + 1) * 64, :]), _up(XN[sl][...]))
            PHQ[i, c * 128:c * 128 + 64, :] = _features(p[0:64, :])
            PHQ[i, c * 128 + 64:(c + 1) * 128, :] = _features(p[64:128, :])
            yield
        for c in range(4):
            p = _dot(_up(WALL[512 + c * 64: 512 + (c + 1) * 64, :]), _up(XN[sl][...]))
            VA[sl][80 * c: 80 * c + 32, :] = _pack2(p[0:32, :], p[32:64, :])
            VA[sl][80 * c + 40: 80 * c + 72, :] = _pack2(p[64:96, :], p[96:128, :])
            yield

    def a1_s3(sl):
        for g in range(8):
            KVA[g] += (_dot_nt(_up(VA[sl][g * 40:(g + 1) * 40, :]),
                               _up(FK[sl][g * 64:(g + 1) * 64, :]))
                       + _dot_nt(_up(VA[sl + 1][g * 40:(g + 1) * 40, :]),
                                 _up(FK[sl + 1][g * 64:(g + 1) * 64, :])))
            yield

    def a_pass1(first, xsrc):
        KVA[...] = jnp.zeros(KVA.shape, F32)
        if first:
            _interleave((_chain(a1_s0(xsrc, 0, 0), a1_s0(xsrc, 2, 2)), 8))
        _interleave((a1_s1(first, xsrc, 0, 0), 12), (a1_s1(first, xsrc, 1, 1), 12))

        def body(jj, carry):
            def blk(sl):
                i = jnp.maximum(4 * jj + sl, 0)
                nxt = jnp.minimum(4 * jj + sl + 2, NT - 2)
                i0 = jnp.minimum(4 * jj + sl + 4, NT - 2)
                p0 = jnp.maximum(4 * jj + sl, -1)

                def run(s3):
                    ex = [(kfft(p0, 2), 4, 0.42, 0.56), (a1_s0(xsrc, i0, sl), 4)] if first else []
                    _interleave(*s3,
                                (_chain(a1_s2(i, sl), a1_s2(i + 1, sl + 1)), 24),
                                (_chain(a1_s1(first, xsrc, nxt, 2 - sl),
                                        a1_s1(first, xsrc, nxt + 1, 3 - sl)), 24), *ex)

                if sl == 0:
                    @pl.when(jj == 0)
                    def _():
                        run([])

                @pl.when(jj > -sl)
                def _():
                    run([(a1_s3(2 - sl), 8)])

            blk(0)
            blk(2)
            return carry

        lax.fori_loop(0, NT // 4, body, 0)
        _interleave((a1_s3(2), 8))
        r = lax.broadcasted_iota(jnp.int32, (40, 128), 0)
        c = lax.broadcasted_iota(jnp.int32, (40, 128), 1)
        msk = (r % 4) == ((c // 2) % 4)
        for g in range(8):
            KVT[g] = _pack2(jnp.where(msk, KVA[g, pl.ds(0, 40, stride=2), :], 0.0),
                            jnp.where(msk, KVA[g, pl.ds(1, 40, stride=2), :], 0.0))

    def a2_s1(i, sl):
        for g in range(8):
            rr = _dot(_up(KVT[g]), _up(PHQ[i, g * 64:(g + 1) * 64, :]))
            rden = 1.0 / (rr[64:72, :] + 1e-6)
            o = (rr[0:64, :].reshape(8, 8, 128) * rden[None]).reshape(64, 128)
            O[sl][g * 32:(g + 1) * 32, :] = _pack2(o[0:32, :], o[32:64, :])
            yield

    def a2_s2(xsrc, i, sl):
        for c in range(4):
            XT[sl][c * 128:(c + 1) * 128, :] = (
                xsrc[i, c * 128:(c + 1) * 128, :]
                + _dot(_up(jnp.concatenate([WOT[g, c * 64:(c + 1) * 64, :] for g in range(4)],
                                           axis=1)), _up(O[sl][...])))
            yield

    def a2_s3(xdst, i, sl):
        def emit(c, w, xe, xo):
            U[i, c * 64:(c + 1) * 64, :] = w
            re = pl.ds(c * 128, 64, stride=2)
            ro = pl.ds(c * 128 + 1, 64, stride=2)
            xdst[i, re, :] = xe + _unpack2(w, 0) * DSK[re, :]
            xdst[i, ro, :] = xo + _unpack2(w, 1) * DSK[ro, :]

        return _ln_gen(lambda c: XT[sl][c * 128:(c + 1) * 128, :],
                       lambda rows: XT[sl][rows, :], emit)

    def a_pass2(xsrc, xdst, first):
        _interleave((a2_s1(0, 0), 8), (a2_s1(1, 1), 8))

        def body(jj, carry):
            def blk(i, sl, prv0, prv1, nxt):
                s1 = [] if nxt is None else [
                    (_chain(a2_s1(nxt, 2 - sl), a2_s1(nxt + 1, 3 - sl)), 16)]
                if first:
                    s1.append((kfft(p0 + 3 * sl, 6), 12) + (KA if sl else KB))
                _interleave((_chain(a2_s3(xdst, prv0, 2 - sl), a2_s3(xdst, prv1, 3 - sl)), 24),
                            (_chain(a2_s2(xsrc, i, sl), a2_s2(xsrc, i + 1, sl + 1)), 8), *s1)

            p0 = jnp.maximum(12 * jj + 16, -6)
            i = 4 * jj
            ia = [jnp.maximum(i, -1), jnp.where(jj == 0, NT, i - 2), jnp.where(jj == 0, NT, i - 1),
                  jnp.maximum(i + 2, -2)]
            ib = [jnp.maximum(i + 2, -3), jnp.maximum(i, -4), jnp.maximum(i + 1, -5),
                  jnp.minimum(i + 4, NT - 2)]

            @pl.when(jj < NT // 4 - 1)
            def _():
                blk(ia[0], 0, *ia[1:])
                blk(ib[0], 2, *ib[1:])

            @pl.when(jj == NT // 4 - 1)
            def _():
                blk(ia[0], 0, *ia[1:])
                blk(ib[0], 2, ib[1], ib[2], None)
            return carry

        lax.fori_loop(0, NT // 4, body, 0)
        _interleave((a2_s3(xdst, NT - 2, 2), 12), (a2_s3(xdst, NT - 1, 3), 12))

    def b_f(j, par):
        rows = pl.ds(pl.multiple_of(j * (RBK // 2), RBK // 2), RBK // 2)
        for n in range(8):
            z0 = _dot(_up(U[n, rows, :]), _up(MF[n]))
            z1 = _dot(_up(U[n + 8, rows, :]), _up(MF[n + 8]))
            ZA[par][n] = z0 + z1
            ZA[par][n + 8] = z0 - z1
            yield

    def b_m(j, par):
        for s in range(RBK // 8):
            rr = pl.ds(s * 8, 8)
            kr = pl.ds(pl.multiple_of(j * RBK + s * 8, 8), 8)
            for h in range(2):
                z = [(ZA[par][8 * h + n, rr, 0:128], ZA[par][8 * h + n, rr, 128:256])
                     for n in range(8)]
                if h:
                    z = [_twiddle(z[n], n, -1) for n in range(8)]
                f = _fft8(z, -1)
                y = [_cmul(f[m], (KF[8 * h + m, kr, 0:128], KF[8 * h + m, kr, 128:256]))
                     for m in range(8)]
                v = _fft8(y, 1)
                if h:
                    v = [_twiddle(v[n], n, 1) for n in range(8)]
                for n in range(8):
                    VB[par][2 * (8 * h + n), rr, :] = v[n][0]
                    VB[par][2 * (8 * h + n) + 1, rr, :] = v[n][1]
                yield

    def b_i(xb, j, vsrc, half=None):
        rs = pl.ds(pl.multiple_of(j * RBK, RBK), RBK)
        ev = pl.ds(0, RBK // 2, stride=2)
        od = pl.ds(1, RBK // 2, stride=2)
        prev = None
        for n in range(8):
            v0, v1 = [], []
            for c in range(2):
                ee, eo = vsrc[2 * n + c, ev, :], vsrc[2 * n + c, od, :]
                oe, oo = vsrc[2 * n + 16 + c, ev, :], vsrc[2 * n + 16 + c, od, :]
                v0.append(_pack2(ee + oe, eo + oo))
                v1.append(_pack2(ee - oe, eo - oo))
            r = [xb[n, rs, :] + _dot_nt(_up(jnp.concatenate(v0, axis=1)), _up(MF[n])),
                 xb[n + 8, rs, :] + _dot_nt(_up(jnp.concatenate(v1, axis=1)), _up(MF[n + 8]))]
            if half is None:
                xb[n, rs, :] = r[0]
                xb[n + 8, rs, :] = r[1]
            elif n % 2:
                for h in range(2):
                    m = n // 2 + 4 * h
                    w = _pack2(prev[h], r[h])
                    if half:
                        w = jnp.concatenate([FK[0][m * RBK:(m + 1) * RBK, :], w], axis=0)
                        xpu[j // 2, pl.ds(m, 128, stride=8), :] = w.T
                    else:
                        FK[0][m * RBK:(m + 1) * RBK, :] = w
            prev = r
            yield

    def b_step(gi, gm, gf):
        for k in range(8):
            if gf is not None:
                next(gf)
            next(gm)
            if gi is not None:
                next(gi)
            next(gm)

    def o_cp(c):
        return pltpu.make_async_copy(
            xpb.at[c], out_hbm.at[:, pl.ds(pl.multiple_of(c * 128, 128), 128)], sem.at[c])

    def b_phase(xb, first):
        _interleave((b_f(0, 0), 8))
        h0, h1 = (None, None) if first else (0, 1)

        def body(jj, carry):
            j = 2 * jj + 1

            @pl.when(jj == 0)
            def _():
                b_step(None, b_m(0, 0), b_f(1, 1))

            @pl.when(jj > 0)
            def _():
                b_step(b_i(xb, jnp.maximum(j - 2, 0), VB[1], h1), b_m(j - 1, 0), b_f(j, 1))
                if not first:
                    o_cp(jj - 1).start()

            @pl.when(jj < NBK // 2 - 1)
            def _():
                b_step(b_i(xb, jnp.maximum(j - 1, 0), VB[0], h0), b_m(j, 1),
                       b_f(jnp.minimum(j + 1, NBK - 1), 0))

            @pl.when(jj == NBK // 2 - 1)
            def _():
                b_step(b_i(xb, NBK - 2, VB[0], h0), b_m(NBK - 1, 1), None)
            return carry

        lax.fori_loop(0, NBK // 2, body, 0)
        _interleave((b_i(xb, NBK - 1, VB[1], h1), 8))

    with jax.named_scope("a1"):
        a_pass1(True, XA)
    with jax.named_scope("a2"):
        a_pass2(XA, XB, True)
    with jax.named_scope("b"):
        b_phase(XB, True)
    with jax.named_scope("a1b"):
        a_pass1(False, XB)
    with jax.named_scope("a2b"):
        a_pass2(XB, XA, False)
    with jax.named_scope("bb"):
        b_phase(XA, False)
    with jax.named_scope("out"):
        o_cp(3).start()
        for c in range(4):
            o_cp(c).wait()


@jax.jit
def pallas_interleave_layers__linear_kernel_hedgehog__ssm_conv_s4__prompt_kernel(
    A_x: jax.Array,
    A_wqkv: jax.Array,
    A_w_phi: jax.Array,
    A_wo: jax.Array,
    B_u: jax.Array,
    B_A_re: jax.Array,
    B_A_im: jax.Array,
    B_B_re: jax.Array,
    B_B_im: jax.Array,
    B_C_re: jax.Array,
    B_C_im: jax.Array,
    B_log_dt: jax.Array,
    B_Dskip: jax.Array,
):
    mf = jnp.asarray(_dft_table())
    vm = pl.BlockSpec(memory_space=pltpu.VMEM)
    hb = pl.BlockSpec(memory_space=pl.ANY)
    out = pl.pallas_call(
        _kernel,
        out_shape=jax.ShapeDtypeStruct((S, D), BF16),
        in_specs=[hb, hb, vm, hb, hb, hb, hb, hb, hb, hb, vm, vm, hb],
        out_specs=hb,
        scratch_shapes=[
            pltpu.VMEM((4, S // 2, 128), U32),
            pltpu.VMEM((12, D // 2, 128), U32),
            pltpu.VMEM((4, 64, D), U32),
            pltpu.VMEM((6, D // 2, NS), U32),
            pltpu.VMEM((NT, 64, 256), U32),
            pltpu.VMEM((NT + 1, D + RBK, 128), F32),
            pltpu.VMEM((NT + 1, D + RBK, 128), F32),
            pltpu.VMEM((NT, D, 256), F32),
            pltpu.VMEM((NT, 512, 128), U32),
            pltpu.VMEM((768, D), U32),
            pltpu.VMEM((4, 256, 128), U32),
            pltpu.VMEM((8, 80, 128), F32),
            pltpu.VMEM((8, 40, 128), U32),
            pltpu.VMEM((2, NHI * 2 * EP, 128), U32),
            pltpu.VMEM((2, NHI * 2 * EP, 128), U32),
            pltpu.VMEM((2, NLO * 2 * EP, 128), U32),
            pltpu.VMEM((2, NLO * 2 * EP, 128), U32),
            pltpu.VMEM((4, D, 128), F32),
            pltpu.VMEM((NHI * 4 * PITCH + 136, 128), F32),
            pltpu.VMEM((D, 128), F32),
            pltpu.VMEM((D, 128), F32),
            pltpu.VMEM((NT + 1, 256, 128), U32),
            pltpu.VMEM((NT, RBK, 256), F32),
            pltpu.VMEM((NT, RBK, 256), F32),
            pltpu.VMEM((2 * NT, RBK, 128), F32),
            pltpu.VMEM((2 * NT, RBK, 128), F32),
            pltpu.VMEM((6, 9, 64, 128), U32),
            pltpu.SemaphoreType.DMA((11,)),
            pltpu.SemaphoreType.DMA((4, 4)),
        ] + [pltpu.VMEM((256, 128), U32)] * 4
          + [pltpu.VMEM((512, 128), U32)] * 4
          + [pltpu.VMEM((320, 128), U32)] * 4
          + [pltpu.VMEM((256, 128), U32)] * 4
          + [pltpu.VMEM((D, 128), F32)] * 4,
        compiler_params=pltpu.CompilerParams(vmem_limit_bytes=110 * 1024 * 1024),
    )(A_x.reshape(S, D), A_wqkv, jnp.transpose(A_w_phi, (1, 2, 0)).reshape(256, 32), A_wo,
      B_A_re, B_A_im, B_B_re, B_B_im, B_C_re, B_C_im,
      B_log_dt, B_Dskip, mf)
    return out.reshape(1, S, D)
```

```python
import numpy as np
import jax
import jax.numpy as jnp
from jax import lax
import jax.experimental.pallas as pl
import jax.experimental.pallas.tpu as pltpu

F32 = jnp.float32
BF16 = jnp.bfloat16
U32 = jnp.uint32

S = 2048
D = 512
NT = 16
NS = 128
LOG2E = 1.4426950408889634

_R1 = [0, 0, 2, 4, 4, 4, 6, 8, 8, 8, 10, 12, 12, 12, 14, 16]
_R2 = [0, 0, 0, 4, 4, 4, 8, 8, 8, 8, 8, 12, 12, 12, 16, 16]
_R3 = [0, 0, 0, 0, 0, 8, 8, 8, 8, 8, 8, 8, 16, 16, 16, 16]
_HI = ([(0, r) for r in range(17)] + [(1, r) for r in (0, 4, 8, 12, 16)]
       + [(2, r) for r in (0, 8, 16)] + [(3, r) for r in (0, 8, 16)])
_HI_IDX = {qr: i for i, qr in enumerate(_HI)}
NHI = len(_HI)
NLO = 32
GB = 16
EP = 2 * GB + 1
PITCH = 129


def _dft_table():
    n1 = np.arange(16, dtype=np.float64)[:, None, None]
    n2 = np.arange(128, dtype=np.float64)[None, :, None]
    k2 = np.arange(128, dtype=np.float64)[None, None, :]
    th = 2.0 * np.pi * (n1 + 16.0 * n2) * (k2 + 0.5) / 4096.0
    tab = np.concatenate([np.cos(th), -np.sin(th)], axis=2).astype(np.float32)
    bits = tab.astype(BF16).view(np.uint16).astype(np.uint32)
    return bits[:, 0::2, :] | (bits[:, 1::2, :] << 16)


def _cmul(a, b):
    return (a[0] * b[0] - a[1] * b[1], a[0] * b[1] + a[1] * b[0])


def _csq(a):
    return (a[0] * a[0] - a[1] * a[1], (a[0] + a[0]) * a[1])


def _sincos(x):
    big = 12582912.0
    kf = x * 0.6366197723675814 + big
    ki = pltpu.bitcast(kf, jnp.int32)
    k = kf - big
    r = x - k * 1.5703125
    r = r - k * 4.837512969970703125e-4
    r = r - k * 7.54978995489188216e-8
    r = jnp.minimum(jnp.maximum(r, -1.0), 1.0)
    z = r * r
    ps = ((-1.9515295891e-4 * z + 8.3321608736e-3) * z - 1.6666654611e-1) * z * r + r
    pc = (((2.443315711809948e-5 * z - 1.388731625493765e-3) * z + 4.166664568298827e-2) * z
          - 0.5) * z + 1.0
    odd = (ki & 1) == 1
    sn = jnp.where(odd, pc, ps)
    cs = jnp.where(odd, ps, pc)
    sgs = (ki & 2) << 30
    sgc = ((ki + 1) & 2) << 30
    sn = pltpu.bitcast(pltpu.bitcast(sn, jnp.int32) ^ sgs, F32)
    cs = pltpu.bitcast(pltpu.bitcast(cs, jnp.int32) ^ sgc, F32)
    return sn, cs


def _bfly4(x0, x1, x2, x3, sgn):
    a = (x0[0] + x2[0], x0[1] + x2[1])
    b = (x0[0] - x2[0], x0[1] - x2[1])
    c = (x1[0] + x3[0], x1[1] + x3[1])
    d = (x1[0] - x3[0], x1[1] - x3[1])
    y0 = (a[0] + c[0], a[1] + c[1])
    y2 = (a[0] - c[0], a[1] - c[1])
    if sgn < 0:
        y1 = (b[0] + d[1], b[1] - d[0])
        y3 = (b[0] - d[1], b[1] + d[0])
    else:
        y1 = (b[0] - d[1], b[1] + d[0])
        y3 = (b[0] + d[1], b[1] - d[0])
    return y0, y1, y2, y3


def _twiddle(x, m, sgn):
    m = m % 16
    if m == 0:
        return x
    if m == 4:
        return (x[1], -x[0]) if sgn < 0 else (-x[1], x[0])
    c = float(np.cos(2 * np.pi * m / 16))
    s = float(sgn * np.sin(2 * np.pi * m / 16))
    if m in (2, 6):
        h = float(np.sqrt(0.5))
        sc = 1.0 if c > 0 else -1.0
        ss = 1.0 if s > 0 else -1.0
        if sc * ss > 0:
            re = x[0] - x[1]
            im = x[0] + x[1]
            return (re * (h * sc), im * (h * sc))
        re = x[0] + x[1]
        im = x[1] - x[0]
        return (re * (h * sc), im * (h * sc))
    return (x[0] * c - x[1] * s, x[0] * s + x[1] * c)


def _fft16(x, sgn):
    t = [[None] * 4 for _ in range(4)]
    for b in range(4):
        y = _bfly4(x[b], x[4 + b], x[8 + b], x[12 + b], sgn)
        for c in range(4):
            t[b][c] = _twiddle(y[c], b * c, sgn)
    out = [None] * 16
    for c in range(4):
        y = _bfly4(t[0][c], t[1][c], t[2][c], t[3][c], sgn)
        for e in range(4):
            out[c + 4 * e] = y[e]
    return out


def _fft8(x, sgn):
    a = [(x[n][0] + x[n + 4][0], x[n][1] + x[n + 4][1]) for n in range(4)]
    b = [_twiddle((x[n][0] - x[n + 4][0], x[n][1] - x[n + 4][1]), 2 * n, sgn) for n in range(4)]
    ya = _bfly4(a[0], a[1], a[2], a[3], sgn)
    yb = _bfly4(b[0], b[1], b[2], b[3], sgn)
    out = [None] * 8
    for m in range(4):
        out[2 * m] = ya[m]
        out[2 * m + 1] = yb[m]
    return out


def _dot(a, b):
    return jnp.dot(a, b, preferred_element_type=F32)


def _dot_nt(a, b):
    return lax.dot_general(a, b, (((1,), (1,)), ((), ())), preferred_element_type=F32)


def _layernorm_t(xt):
    m = jnp.sum(xt, axis=0, keepdims=True) * (1.0 / D)
    xc = xt - m
    v = jnp.sum(xc * xc, axis=0, keepdims=True) * (1.0 / D)
    return xc * lax.rsqrt(v + 1e-5)


def _pk(x):
    return pltpu.bitcast(x, U32)


def _up(w):
    return pltpu.bitcast(w, BF16)


def _pack2(a, b):
    return pltpu.pack_elementwise([a, b], packed_dtype=BF16)


def _unpack2(w, i):
    return pltpu.unpack_elementwise(w, index=i, packed_dtype=BF16, unpacked_dtype=F32)


def _features(p):
    p3 = p.reshape(8, 8, 128)
    mx = jnp.max(p3, axis=0)
    mx = jnp.maximum(mx, pltpu.roll(mx, 4, 0))
    mn = jnp.min(p3, axis=0)
    mn = jnp.minimum(mn, pltpu.roll(mn, 4, 0))
    ep = jnp.exp2(p3 - mx[None])
    en = jnp.exp2(mn[None] - p3)
    sp = jnp.sum(ep, axis=0)
    sn = jnp.sum(en, axis=0)
    rp = 1.0 / (sp + pltpu.roll(sp, 4, 0))
    rn = 1.0 / (sn + pltpu.roll(sn, 4, 0))
    return _pack2((ep * rp[None]).reshape(64, 128), (en * rn[None]).reshape(64, 128))


def _interleave(*stages):
    order = []
    for i, st in enumerate(stages):
        lo, hi = st[2:] if len(st) > 2 else (0.0, 1.0)
        order += [(lo + (hi - lo) * (k + 0.5) / st[1], i) for k in range(st[1])]
    for _, i in sorted(order):
        next(stages[i][0], None)
    for st in stages:
        for _ in st[0]:
            pass


def _colsum8(x):
    return jnp.sum(x.reshape(x.shape[0] // 8, 8, 128), axis=0)


def _ln_gen(first_pass, load, emit):
    s = None
    for c in range(4):
        t = _colsum8(first_pass(c))
        s = t if s is None else s + t
        yield
    m = jnp.sum(s, axis=0, keepdims=True) * (1.0 / D)
    v = None
    for c in range(4):
        xc = load(pl.ds(c * 128, 128)) - m
        t = _colsum8(xc * xc)
        v = t if v is None else v + t
        yield
    r = lax.rsqrt(jnp.sum(v, axis=0, keepdims=True) * (1.0 / D) + 1e-5)
    for c in range(4):
        xe = load(pl.ds(c * 128, 64, stride=2))
        xo = load(pl.ds(c * 128 + 1, 64, stride=2))
        emit(c, _pack2((xe - m) * r, (xo - m) * r), xe, xo)
        yield


MME = 1.0
KB = (0.0, 1.0)
KA = (0.0, 1.0)
ES = 0.0
RBK = 64
NBK = D // RBK


def _kernel(x_hbm, wqkv_hbm, wphi_ref, wo_hbm, are_hbm, aim_hbm, bre_hbm, bim_hbm,
            cre_hbm, cim_hbm, ldt_ref, dsk_ref, mf_hbm, out_hbm,
            XP, WQ, WO, SSM, MF, XA, XB, KF, PHQ, WALL, WOT, KVA, KVT, EH0, EH1, EL0, EL1, EW, KS, DSK, DT,
            U, ZA0, ZA1, VB0, VB1, BD, sem, wsem, *bufs):
    XN, FK, VA, O, XT = [bufs[4 * k:4 * k + 4] for k in range(5)]
    VB = (VB0, VB1)
    ZA = (ZA0, ZA1)
    EHS, ELS = (EH0, EH1), (EL0, EL1)
    lane128 = lax.broadcasted_iota(jnp.int32, (128, 128), 1)
    row128 = lax.broadcasted_iota(jnp.int32, (128, 128), 0)

    ssm_cp = [pltpu.make_async_copy(h.at[pl.ds(hf * 256, 256), :],
                                    SSM.bitcast(BF16).at[k, pl.ds(hf * 256, 256), :],
                                    sem.at[k + 11 * hf])
              for hf in range(2)
              for k, h in enumerate((are_hbm, aim_hbm, bre_hbm, bim_hbm, cre_hbm, cim_hbm))]
    mf_cp = pltpu.make_async_copy(mf_hbm, MF, sem.at[6])
    wqb, wob = WQ.bitcast(BF16), WO.bitcast(BF16)

    def w_cp(g):
        off = pl.multiple_of(g * 128, 128)
        return [pltpu.make_async_copy(wqkv_hbm.at[:, pl.ds(p * D + off, 128)], wqb.at[4 * p + g],
                                      wsem.at[g, p]) for p in range(3)]

    wo_cp = [pltpu.make_async_copy(wo_hbm.at[pl.ds(g * 128, 128), :], wob.at[g], wsem.at[g, 3])
             for g in range(4)]
    xpb = XP.bitcast(BF16)
    x_cp = [pltpu.make_async_copy(x_hbm.at[:, pl.ds(c * 128, 128)], xpb.at[c], sem.at[7 + c])
            for c in range(4)]
    for cp in ssm_cp + wo_cp + w_cp(0):
        cp.start()

    with jax.named_scope("kgen_e"):
        dtb = jnp.exp(ldt_ref[...].reshape(1, D).astype(F32)).astype(BF16).astype(F32)
        DT[...] = jnp.broadcast_to(dtb, (128, D)).T
        DSK[...] = jnp.broadcast_to(dsk_ref[...].reshape(1, D).astype(F32), (128, D)).T

        def hd_fe(f):
            return (f // 64) * 4 + f % 4, 2 * ((f % 64) // 8) + (f % 8) // 4

        hd, fe = hd_fe(2 * (row128 % 64) + row128 // 64)
        t = _pk(jnp.where((lane128 // 16 == hd) & (lane128 % 16 == fe), 1.0, 0.0).astype(BF16))
        for k in range(2, 6):
            BD[k, 4] = t
        r256 = lax.broadcasted_iota(jnp.int32, (128, 256), 0)
        c256 = lax.broadcasted_iota(jnp.int32, (128, 256), 1)
        e2t = jnp.where(c256 % 16 == hd_fe(2 * (r256 % 64) + r256 // 64)[1], 1.0, 0.0).astype(BF16)
        hsel = (lax.broadcasted_iota(jnp.int32, (128, 32), 1)
                - lax.broadcasted_iota(jnp.int32, (128, 32), 0) // 16)
        for g in range(4):
            z = _dot_nt(jnp.where(hsel == 8 * g, 1.0, 0.0).astype(BF16), wphi_ref[...])
            z = jnp.where(c256 // 16 == r256 % 16, z, 0.0).astype(BF16)
            t = _pk(jnp.where(lane128 // 16 == hd, _dot_nt(e2t, z), 0.0).astype(BF16))
            for k in range(6):
                BD[k, g] = t
        k6 = lane128 % 64
        r6 = 32 * (k6 % 2) + k6 // 2
        a6 = 32 * (r6 % 2) + r6 // 2
        t = _pk(jnp.where(((row128 // 16) == (lane128 // 64) * 4 + a6 % 4)
                          & (row128 % 16 == 2 * (a6 // 8) + (a6 % 8) // 4), 1.0, 0.0).astype(BF16))
        for k in range(16):
            BD[k // 4, 5 + k % 4] = t
        for b in range(4):
            VA[b][...] = jnp.full(VA[b].shape, 0x3F803F80, U32)
        for cp in ssm_cp[:6]:
            cp.wait()


    with jax.named_scope("kgen_e1"):
        def e1body(i, carry):
            hr = pl.ds(pl.multiple_of(i * 16, 16), 16)
            raw = [SSM[k, hr, :] for k in range(6)]
            for par in range(2):
                dt = DT[pl.ds(i * 32 + par, 16, stride=2), :]
                prm = [_unpack2(raw[k], par) for k in range(6)]
                dts = dt * (2.0 / 4096.0)
                c0 = _cmul((prm[4], prm[5]), (dts * prm[2], dts * prm[3]))
                mag = jnp.exp(dt * prm[0])
                sn, cs = _sincos(dt * prm[1])
                for k, v in enumerate((mag * cs, mag * sn, c0[0], c0[1])):
                    for h in range(2):
                        EW[k, pl.ds(pl.multiple_of(i * 32 + 16 * h + 8 * par, 8), 8), :] = (
                            v[8 * h:8 * h + 8, :])
            return carry

        lax.fori_loop(0, D // 64, e1body, 0)
        for cp in ssm_cp[6:]:
            cp.wait()
        for cp in w_cp(1) + w_cp(2) + w_cp(3) + x_cp + [mf_cp]:
            cp.start()
        lax.fori_loop(D // 64, D // 32, e1body, 0)

    def e_piece(blk, dd, hf, par):
        rows = pl.ds(pl.multiple_of(dd * 128 + blk * GB + 8 * hf, 8), 8)
        EH, EL = EHS[par], ELS[par]
        w = {1: (EW[0, rows, :], EW[1, rows, :])}
        c = {}

        def put(ref, n, k, u, v):
            rr = pl.ds((dd * n + k) * EP + 16 * hf, 8, stride=2)
            for cc in range(2):
                ref[cc, rr, :] = _pack2(u[cc], v[cc])

        for b in (1, 2, 4, 8, 16, 32):
            w[2 * b] = _csq(w[b])
        lo = {0: (jnp.ones((8, 128), F32), jnp.zeros((8, 128), F32)), 1: w[16], 2: w[32],
              3: _cmul(w[16], w[32]), 4: w[64]}
        for j in range(NLO):
            if j > 4:
                lo[j] = _cmul(lo[j - 4], w[64])
            if j % 2:
                put(EL, NLO // 2, j // 2, lo[j - 1], lo[j])
            if j % 8 == 7:
                yield
        w[512] = _cmul(lo[28], w[64])
        w[1024] = _csq(w[512])
        w[1536] = _cmul(w[1024], w[512])
        c[0] = (EW[2, rows, :], EW[3, rows, :])
        for r in range(1, 17):
            c[r] = (_cmul(c[r - 4], w[4]) if r >= 4 else
                    _cmul(c[1], w[2]) if r == 3 else _cmul(c[0], w[r]))
            if r % 2:
                put(EH, NHI // 2, r // 2, c[r - 1], c[r])
            if r % 8 == 7:
                yield
        hi = [c[r] if q == 0 else _cmul(c[r], w[512 * q]) for q, r in _HI[16:]]
        for k in range(6):
            put(EH, NHI // 2, 8 + k, hi[2 * k], hi[2 * k + 1])
        yield

    def e_blk(blk, par):
        for hf in range(GB // 8):
            for dd in range(4):
                yield from e_piece(blk, dd, hf, par)

    def mm_blk(blk, par):
        for g in range(GB):
            t = [_dot_nt(_up(EHS[par][c, pl.ds(2 * g, NHI * 2, stride=EP), :]),
                         _up(ELS[par][c, pl.ds(2 * g, NLO * 2, stride=EP), :])) for c in range(2)]
            KS[pl.ds(2 * GB * blk + 2 * g, NHI * 4, stride=PITCH), :] = t[0] - t[1]
            yield

    def wprep(g, parts):
        for q in parts:
            p, c = divmod(q, 4)
            if True:
                if p < 3:
                    t = _dot_nt(_up(BD[q % 6, g] if p < 2 else BD[q % 6, 4]),
                                _up(WQ[4 * p + g, c * 64:(c + 1) * 64, :]))
                    if p < 2:
                        t = t * LOG2E
                    WALL[pl.ds(pl.multiple_of(p * 256 + g * 64, 64), 64),
                         c * 128:(c + 1) * 128] = _pack2(t[0:64, :], t[64:128, :])
                else:
                    wot = _up(WO[g, :, c * 128:(c + 1) * 128]).astype(F32).T.astype(BF16)
                    WOT[g, c * 64:(c + 1) * 64, :] = _pk(_dot(wot, _up(BD[g, 5 + c])).astype(BF16))
                yield

    def _chain(*gens):
        for g in gens:
            yield from g

    with jax.named_scope("kgen_e2"):
        _interleave((_chain(*[e_piece(0, dd, 0, 0) for dd in range(4)]), 28))
        for cp in wo_cp:
            cp.wait()
        _interleave((_chain(*[e_piece(0, dd, 1, 0) for dd in range(4)]), 28),
                    (_chain(*[wprep(g, range(12, 16)) for g in range(4)]), 16))

        def ebody(jj, carry):
            for cp in w_cp(jj):
                cp.wait()
            im = [jnp.maximum(2 * jj + k, -1) for k in range(2)]
            ie = [jnp.maximum(2 * jj + 1, -2), jnp.minimum(2 * jj + 2, 128 // GB - 1)]
            iw = jnp.maximum(jj, -3)

            @pl.when(jj >= -1)
            def _():
                _interleave((mm_blk(im[0], 0), GB, 0.0, MME), (e_blk(ie[0], 1), 28 * GB // 8, ES, 1.0),
                            (wprep(iw, range(0, 6)), 6, 0.0, MME))

            @pl.when(jj < 64 // GB - 1)
            def _():
                _interleave((mm_blk(im[1], 1), GB, 0.0, MME), (e_blk(ie[1], 0), 28 * GB // 8, ES, 1.0),
                            (wprep(iw, range(6, 12)), 6, 0.0, MME))

            @pl.when(jj == 64 // GB - 1)
            def _():
                _interleave((mm_blk(im[1], 1), GB), (wprep(iw, range(6, 12)), 6))
            return carry

        lax.fori_loop(0, 64 // GB, ebody, 0)

    with jax.named_scope("kgen_asm"):
        mf_cp.wait()
        def rolls(dd):
            for idx, (q, r) in enumerate(_HI):
                sh = ((q - dd) * 32) % 128
                if sh:
                    sl = pl.ds((dd * NHI + idx) * PITCH, 128, stride=2)
                    KS[sl, :] = pltpu.roll(KS[sl, :], sh, 1)
                    yield

        def slab(q, r, dd):
            return KS[pl.ds((dd * NHI + _HI_IDX[(q, r)]) * PITCH, 128, stride=2), :]

        def kpart(n1, dd):
            t = jnp.where(lane128 < 96, slab(2, _R3[n1], dd), slab(3, _R3[n1], dd))
            t = jnp.where(lane128 < 64, slab(1, _R2[n1], dd), t)
            t = jnp.where(lane128 < 32, slab(0, _R1[n1], dd), t)
            t = jnp.where(lane128 < 16, slab(0, n1, dd), t)
            t = t.reshape(8, 16, 128)
            return _dot(_up(_pack2(t[:, 0:8, :], t[:, 8:16, :]).reshape(64, 128)), _up(MF[n1]))

        def asm(dd):
            for n1 in range(8):
                z0, z1 = kpart(n1, dd), kpart(n1 + 8, dd)
                KF[n1, dd * 128:(dd + 1) * 128, :] = z0 + z1
                KF[n1 + 8, dd * 128:(dd + 1) * 128, :] = z0 - z1
                yield

        _interleave((rolls(0), 11))
        for dd in range(4):
            _interleave((asm(dd), 8), *([(rolls(dd + 1), 25)] if dd < 3 else []))

    def kfft(p0, n):
        for k in range(n):
            rows = pl.ds(pl.multiple_of((p0 + k) * 8, 8), 8)
            for h in range(2):
                z = [(KF[8 * h + j, rows, 0:128], KF[8 * h + j, rows, 128:256]) for j in range(8)]
                if h:
                    z = [_twiddle(z[j], j, -1) for j in range(8)]
                f = _fft8(z, -1)
                for j in range(8):
                    KF[8 * h + j, rows, 0:128] = f[j][0]
                    KF[8 * h + j, rows, 128:256] = f[j][1]
                yield

    for cp in x_cp:
        cp.wait()

    xpu = XP

    def a1_s0(xsrc, i, sl):
        for c in range(4):
            w = xpu[c, pl.ds(i // 2, 128, stride=8), :].T
            for par in range(2):
                XT[sl + par][c * 128:(c + 1) * 128, :] = _unpack2(w, par)
            yield

    def a1_s1(first, xsrc, i, sl):
        def emit(c, w, xe, xo):
            XN[sl][c * 64:(c + 1) * 64, :] = w

        load = (lambda rows: XT[sl][rows, :]) if first else (lambda rows: xsrc[i, rows, :])

        def fp(c):
            xt = load(pl.ds(c * 128, 128))
            if first:
                xsrc[i, c * 128:(c + 1) * 128, :] = xt
            return xt

        return _ln_gen(fp, load, emit)

    def a1_s2(i, sl):
        for c in range(4):
            p = _dot(_up(WALL[256 + c * 64: 256 + (c + 1) * 64, :]), _up(XN[sl][...]))
            FK[sl][c * 128:c * 128 + 64, :] = _features(p[0:64, :])
            FK[sl][c * 128 + 64:(c + 1) * 128, :] = _features(p[64:128, :])
            yield
        for c in range(4):
            p = _dot(_up(WALL[c * 64:(c + 1) * 64, :]), _up(XN[sl][...]))
            PHQ[i, c * 128:c * 128 + 64, :] = _features(p[0:64, :])
            PHQ[i, c * 128 + 64:(c + 1) * 128, :] = _features(p[64:128, :])
            yield
        for c in range(4):
            p = _dot(_up(WALL[512 + c * 64: 512 + (c + 1) * 64, :]), _up(XN[sl][...]))
            VA[sl][80 * c: 80 * c + 32, :] = _pack2(p[0:32, :], p[32:64, :])
            VA[sl][80 * c + 40: 80 * c + 72, :] = _pack2(p[64:96, :], p[96:128, :])
            yield

    def a1_s3(sl):
        for g in range(8):
            KVA[g] += (_dot_nt(_up(VA[sl][g * 40:(g + 1) * 40, :]),
                               _up(FK[sl][g * 64:(g + 1) * 64, :]))
                       + _dot_nt(_up(VA[sl + 1][g * 40:(g + 1) * 40, :]),
                                 _up(FK[sl + 1][g * 64:(g + 1) * 64, :])))
            yield

    def a_pass1(first, xsrc):
        KVA[...] = jnp.zeros(KVA.shape, F32)
        if first:
            _interleave((_chain(a1_s0(xsrc, 0, 0), a1_s0(xsrc, 2, 2)), 8))
        _interleave((a1_s1(first, xsrc, 0, 0), 12), (a1_s1(first, xsrc, 1, 1), 12))

        def body(jj, carry):
            def blk(sl):
                i = jnp.maximum(4 * jj + sl, 0)
                nxt = jnp.minimum(4 * jj + sl + 2, NT - 2)
                i0 = jnp.minimum(4 * jj + sl + 4, NT - 2)
                p0 = jnp.maximum(4 * jj + sl, -1)

                def run(s3):
                    ex = [(kfft(p0, 2), 4, 0.42, 0.56), (a1_s0(xsrc, i0, sl), 4)] if first else []
                    _interleave(*s3,
                                (_chain(a1_s2(i, sl), a1_s2(i + 1, sl + 1)), 24),
                                (_chain(a1_s1(first, xsrc, nxt, 2 - sl),
                                        a1_s1(first, xsrc, nxt + 1, 3 - sl)), 24), *ex)

                if sl == 0:
                    @pl.when(jj == 0)
                    def _():
                        run([])

                @pl.when(jj > -sl)
                def _():
                    run([(a1_s3(2 - sl), 8)])

            blk(0)
            blk(2)
            return carry

        lax.fori_loop(0, NT // 4, body, 0)
        _interleave((a1_s3(2), 8))
        r = lax.broadcasted_iota(jnp.int32, (40, 128), 0)
        c = lax.broadcasted_iota(jnp.int32, (40, 128), 1)
        msk = (r % 4) == ((c // 2) % 4)
        for g in range(8):
            KVT[g] = _pack2(jnp.where(msk, KVA[g, pl.ds(0, 40, stride=2), :], 0.0),
                            jnp.where(msk, KVA[g, pl.ds(1, 40, stride=2), :], 0.0))

    def a2_s1(i, sl):
        for g in range(8):
            rr = _dot(_up(KVT[g]), _up(PHQ[i, g * 64:(g + 1) * 64, :]))
            rden = 1.0 / (rr[64:72, :] + 1e-6)
            o = (rr[0:64, :].reshape(8, 8, 128) * rden[None]).reshape(64, 128)
            O[sl][g * 32:(g + 1) * 32, :] = _pack2(o[0:32, :], o[32:64, :])
            yield

    def a2_s2(xsrc, i, sl):
        for c in range(4):
            XT[sl][c * 128:(c + 1) * 128, :] = (
                xsrc[i, c * 128:(c + 1) * 128, :]
                + _dot(_up(jnp.concatenate([WOT[g, c * 64:(c + 1) * 64, :] for g in range(4)],
                                           axis=1)), _up(O[sl][...])))
            yield

    def a2_s3(xdst, i, sl):
        def emit(c, w, xe, xo):
            U[i, c * 64:(c + 1) * 64, :] = w
            re = pl.ds(c * 128, 64, stride=2)
            ro = pl.ds(c * 128 + 1, 64, stride=2)
            xdst[i, re, :] = xe + _unpack2(w, 0) * DSK[re, :]
            xdst[i, ro, :] = xo + _unpack2(w, 1) * DSK[ro, :]

        return _ln_gen(lambda c: XT[sl][c * 128:(c + 1) * 128, :],
                       lambda rows: XT[sl][rows, :], emit)

    def a_pass2(xsrc, xdst, first):
        _interleave((a2_s1(0, 0), 8), (a2_s1(1, 1), 8))

        def body(jj, carry):
            def blk(i, sl, prv0, prv1, nxt):
                s1 = [] if nxt is None else [
                    (_chain(a2_s1(nxt, 2 - sl), a2_s1(nxt + 1, 3 - sl)), 16)]
                if first:
                    s1.append((kfft(p0 + 3 * sl, 6), 12) + (KA if sl else KB))
                _interleave((_chain(a2_s3(xdst, prv0, 2 - sl), a2_s3(xdst, prv1, 3 - sl)), 24),
                            (_chain(a2_s2(xsrc, i, sl), a2_s2(xsrc, i + 1, sl + 1)), 8), *s1)

            p0 = jnp.maximum(12 * jj + 16, -6)
            i = 4 * jj
            ia = [jnp.maximum(i, -1), jnp.where(jj == 0, NT, i - 2), jnp.where(jj == 0, NT, i - 1),
                  jnp.maximum(i + 2, -2)]
            ib = [jnp.maximum(i + 2, -3), jnp.maximum(i, -4), jnp.maximum(i + 1, -5),
                  jnp.minimum(i + 4, NT - 2)]

            @pl.when(jj < NT // 4 - 1)
            def _():
                blk(ia[0], 0, *ia[1:])
                blk(ib[0], 2, *ib[1:])

            @pl.when(jj == NT // 4 - 1)
            def _():
                blk(ia[0], 0, *ia[1:])
                blk(ib[0], 2, ib[1], ib[2], None)
            return carry

        lax.fori_loop(0, NT // 4, body, 0)
        _interleave((a2_s3(xdst, NT - 2, 2), 12), (a2_s3(xdst, NT - 1, 3), 12))

    def b_f(j, par):
        rows = pl.ds(pl.multiple_of(j * (RBK // 2), RBK // 2), RBK // 2)
        for n in range(8):
            z0 = _dot(_up(U[n, rows, :]), _up(MF[n]))
            z1 = _dot(_up(U[n + 8, rows, :]), _up(MF[n + 8]))
            ZA[par][n] = z0 + z1
            ZA[par][n + 8] = z0 - z1
            yield

    def b_m(j, par):
        for s in range(RBK // 8):
            rr = pl.ds(s * 8, 8)
            kr = pl.ds(pl.multiple_of(j * RBK + s * 8, 8), 8)
            for h in range(2):
                z = [(ZA[par][8 * h + n, rr, 0:128], ZA[par][8 * h + n, rr, 128:256])
                     for n in range(8)]
                if h:
                    z = [_twiddle(z[n], n, -1) for n in range(8)]
                f = _fft8(z, -1)
                y = [_cmul(f[m], (KF[8 * h + m, kr, 0:128], KF[8 * h + m, kr, 128:256]))
                     for m in range(8)]
                v = _fft8(y, 1)
                if h:
                    v = [_twiddle(v[n], n, 1) for n in range(8)]
                for n in range(8):
                    VB[par][2 * (8 * h + n), rr, :] = v[n][0]
                    VB[par][2 * (8 * h + n) + 1, rr, :] = v[n][1]
                yield

    def b_i(xb, j, vsrc, half=None):
        rs = pl.ds(pl.multiple_of(j * RBK, RBK), RBK)
        ev = pl.ds(0, RBK // 2, stride=2)
        od = pl.ds(1, RBK // 2, stride=2)
        prev = None
        for n in range(8):
            v0, v1 = [], []
            for c in range(2):
                ee, eo = vsrc[2 * n + c, ev, :], vsrc[2 * n + c, od, :]
                oe, oo = vsrc[2 * n + 16 + c, ev, :], vsrc[2 * n + 16 + c, od, :]
                v0.append(_pack2(ee + oe, eo + oo))
                v1.append(_pack2(ee - oe, eo - oo))
            r = [xb[n, rs, :] + _dot_nt(_up(jnp.concatenate(v0, axis=1)), _up(MF[n])),
                 xb[n + 8, rs, :] + _dot_nt(_up(jnp.concatenate(v1, axis=1)), _up(MF[n + 8]))]
            if half is None:
                xb[n, rs, :] = r[0]
                xb[n + 8, rs, :] = r[1]
            elif n % 2:
                for h in range(2):
                    m = n // 2 + 4 * h
                    w = _pack2(prev[h], r[h])
                    if half:
                        w = jnp.concatenate([FK[0][m * RBK:(m + 1) * RBK, :], w], axis=0)
                        xpu[j // 2, pl.ds(m, 128, stride=8), :] = w.T
                    else:
                        FK[0][m * RBK:(m + 1) * RBK, :] = w
            prev = r
            yield

    def b_step(gi, gm, gf):
        for k in range(8):
            if gf is not None:
                next(gf)
            next(gm)
            if gi is not None:
                next(gi)
            next(gm)

    def o_cp(c):
        return pltpu.make_async_copy(
            xpb.at[c], out_hbm.at[:, pl.ds(pl.multiple_of(c * 128, 128), 128)], sem.at[c])

    def b_phase(xb, first):
        _interleave((b_f(0, 0), 8))
        h0, h1 = (None, None) if first else (0, 1)

        def body(jj, carry):
            j = 2 * jj + 1

            @pl.when(jj == 0)
            def _():
                b_step(None, b_m(0, 0), b_f(1, 1))

            @pl.when(jj > 0)
            def _():
                b_step(b_i(xb, jnp.maximum(j - 2, 0), VB[1], h1), b_m(j - 1, 0), b_f(j, 1))
                if not first:
                    o_cp(jj - 1).start()

            @pl.when(jj < NBK // 2 - 1)
            def _():
                b_step(b_i(xb, jnp.maximum(j - 1, 0), VB[0], h0), b_m(j, 1),
                       b_f(jnp.minimum(j + 1, NBK - 1), 0))

            @pl.when(jj == NBK // 2 - 1)
            def _():
                b_step(b_i(xb, NBK - 2, VB[0], h0), b_m(NBK - 1, 1), None)
            return carry

        lax.fori_loop(0, NBK // 2, body, 0)
        _interleave((b_i(xb, NBK - 1, VB[1], h1), 8))

    with jax.named_scope("a1"):
        a_pass1(True, XA)
    with jax.named_scope("a2"):
        a_pass2(XA, XB, True)
    with jax.named_scope("b"):
        b_phase(XB, True)
    with jax.named_scope("a1b"):
        a_pass1(False, XB)
    with jax.named_scope("a2b"):
        a_pass2(XB, XA, False)
    with jax.named_scope("bb"):
        b_phase(XA, False)
    with jax.named_scope("out"):
        o_cp(3).start()
        for c in range(4):
            o_cp(c).wait()


@jax.jit
def pallas_interleave_layers__linear_kernel_hedgehog__ssm_conv_s4__prompt_kernel(
    A_x: jax.Array,
    A_wqkv: jax.Array,
    A_w_phi: jax.Array,
    A_wo: jax.Array,
    B_u: jax.Array,
    B_A_re: jax.Array,
    B_A_im: jax.Array,
    B_B_re: jax.Array,
    B_B_im: jax.Array,
    B_C_re: jax.Array,
    B_C_im: jax.Array,
    B_log_dt: jax.Array,
    B_Dskip: jax.Array,
):
    mf = jnp.asarray(_dft_table())
    vm = pl.BlockSpec(memory_space=pltpu.VMEM)
    hb = pl.BlockSpec(memory_space=pl.ANY)
    out = pl.pallas_call(
        _kernel,
        out_shape=jax.ShapeDtypeStruct((S, D), BF16),
        in_specs=[hb, hb, vm, hb, hb, hb, hb, hb, hb, hb, vm, vm, hb],
        out_specs=hb,
        scratch_shapes=[
            pltpu.VMEM((4, S // 2, 128), U32),
            pltpu.VMEM((12, D // 2, 128), U32),
            pltpu.VMEM((4, 64, D), U32),
            pltpu.VMEM((6, D // 2, NS), U32),
            pltpu.VMEM((NT, 64, 256), U32),
            pltpu.VMEM((NT + 1, D + RBK, 128), F32),
            pltpu.VMEM((NT + 1, D + RBK, 128), F32),
            pltpu.VMEM((NT, D, 256), F32),
            pltpu.VMEM((NT, 512, 128), U32),
            pltpu.VMEM((768, D), U32),
            pltpu.VMEM((4, 256, 128), U32),
            pltpu.VMEM((8, 80, 128), F32),
            pltpu.VMEM((8, 40, 128), U32),
            pltpu.VMEM((2, NHI * 2 * EP, 128), U32),
            pltpu.VMEM((2, NHI * 2 * EP, 128), U32),
            pltpu.VMEM((2, NLO * 2 * EP, 128), U32),
            pltpu.VMEM((2, NLO * 2 * EP, 128), U32),
            pltpu.VMEM((4, D, 128), F32),
            pltpu.VMEM((NHI * 4 * PITCH + 136, 128), F32),
            pltpu.VMEM((D, 128), F32),
            pltpu.VMEM((D, 128), F32),
            pltpu.VMEM((NT + 1, 256, 128), U32),
            pltpu.VMEM((NT, RBK, 256), F32),
            pltpu.VMEM((NT, RBK, 256), F32),
            pltpu.VMEM((2 * NT, RBK, 128), F32),
            pltpu.VMEM((2 * NT, RBK, 128), F32),
            pltpu.VMEM((6, 9, 64, 128), U32),
            pltpu.SemaphoreType.DMA((17,)),
            pltpu.SemaphoreType.DMA((4, 4)),
        ] + [pltpu.VMEM((256, 128), U32)] * 4
          + [pltpu.VMEM((512, 128), U32)] * 4
          + [pltpu.VMEM((320, 128), U32)] * 4
          + [pltpu.VMEM((256, 128), U32)] * 4
          + [pltpu.VMEM((D, 128), F32)] * 4,
        compiler_params=pltpu.CompilerParams(vmem_limit_bytes=110 * 1024 * 1024),
    )(A_x.reshape(S, D), A_wqkv, jnp.transpose(A_w_phi, (1, 2, 0)).reshape(256, 32), A_wo,
      B_A_re, B_A_im, B_B_re, B_B_im, B_C_re, B_C_im,
      B_log_dt, B_Dskip, mf)
    return out.reshape(1, S, D)
```
